```python
import jax
import jax.numpy as jnp

def _softmax(x, axis=-1):
    return jax.nn.softmax(x, axis=axis)

def _gelu(x):
    return jax.nn.gelu(x, approximate=True)

def _silu(x):
    return jax.nn.silu(x)

def _sigmoid(x):
    return jax.nn.sigmoid(x)

def _layernorm(x, axis=-1, eps=1e-05):
    m = jnp.mean(x, axis=axis, keepdims=True)
    v = jnp.var(x, axis=axis, keepdims=True)
    return (x - m) / jnp.sqrt(v + eps)

def _scatter_add(tgt, idx, src, axis=0):
    return tgt.at[idx].add(src)

def _segment_sum(src, seg, n):
    return jax.ops.segment_sum(src, seg, n)

class _Rng:

    def __init__(self, key):
        self._k = key

    def _next(self):
        self._k, sub = jax.random.split(self._k)
        return sub

    def normal(self, shape):
        return jax.random.normal(self._next(), shape, dtype=jnp.bfloat16)

    def randint(self, lo, hi, shape):
        return jax.random.randint(self._next(), shape, lo, hi, dtype=jnp.int32)

    def uniform(self, shape, lo=0.0, hi=1.0):
        return jax.random.uniform(self._next(), shape, jnp.bfloat16, lo, hi)

    def permutation(self, n):
        return jax.random.permutation(self._next(), n)
kernel_name = 'concat_heads__sliding_local_dilated__memory_aug_recurrent_mem_tr__prompt'

def setup_inputs():
    _rng = _Rng(jax.random.key(int.from_bytes(__import__("os").urandom(4), "little")))
    _w = lambda a: (lambda t: t.astype(jnp.bfloat16) if jnp.issubdtype(t.dtype, jnp.floating) else t)(jnp.asarray(a))

    def _A_setup():
        B, S, D = (1, 2048, 640)
        return {'x': _w((lambda *s: _rng.normal(s) * 0.05)(B, S, D)), 'wqkv': _w((lambda *s: _rng.normal(s) * 0.05)(D, 3 * D)), 'wo': _w((lambda *s: _rng.normal(s) * 0.05)(D, D))}
    _A_in = _A_setup()

    def _B_setup():
        B, S, Dm = (1, 2048, 640)
        H, Dh = (32, 192)
        M, seg = (8, 32)
        seg = min(seg, S)
        S = S // seg * seg
        return {'x': _w((lambda *s: _rng.normal(s) * 0.05)(B, S, Dm)), 'mem0': _w((lambda *s: _rng.normal(s) * 0.05)(B, M, Dm)), 'Wq': _w((lambda *s: _rng.normal(s) * 0.05)(Dm, H, Dh) * Dm ** (-0.5)), 'Wk': _w((lambda *s: _rng.normal(s) * 0.05)(Dm, H, Dh) * Dm ** (-0.5)), 'Wv': _w((lambda *s: _rng.normal(s) * 0.05)(Dm, H, Dh) * Dm ** (-0.5)), 'Wo': _w((lambda *s: _rng.normal(s) * 0.05)(H, Dh, Dm) * (H * Dh) ** (-0.5)), 'seg_len': seg}
    _B_in = _B_setup()
    return {'A_x': _A_in['x'], 'A_wqkv': _A_in['wqkv'], 'A_wo': _A_in['wo'], 'B_x': _B_in['x'], 'B_mem0': _B_in['mem0'], 'B_Wq': _B_in['Wq'], 'B_Wk': _B_in['Wk'], 'B_Wv': _B_in['Wv'], 'B_Wo': _B_in['Wo'], 'B_seg_len': _B_in['seg_len']}

def reference(A_x, A_wqkv, A_wo, B_x, B_mem0, B_Wq, B_Wk, B_Wv, B_Wo, B_seg_len):

    def _A_ref(x, wqkv, wo):
        B, S, D = x.shape
        H = 32
        Dh = D // H
        W, dil = (8, 2)
        qkv = (lambda x, *d: x.transpose(*d))((x @ wqkv).reshape(B, S, 3, H, Dh), 2, 0, 3, 1, 4)
        q, k, v = (qkv[0], qkv[1], qkv[2])
        scale = Dh ** (-0.5)
        pos = jnp.arange(S)
        off = jnp.arange(W) * dil
        idx = pos[:, None] - off[None, :]
        mask = idx >= 0
        idx_c = jnp.where(mask, idx, 0).reshape(-1)
        kg = k[:, :, idx_c, :].reshape(B, H, S, W, Dh)
        vg = v[:, :, idx_c, :].reshape(B, H, S, W, Dh)
        logits = jnp.einsum('bhsd,bhswd->bhsw', q, kg) * scale
        logits = jnp.where(mask[None, None, :, :], logits, -1000000000.0)
        attn = _softmax(logits, axis=-1)
        o = jnp.einsum('bhsw,bhswd->bhsd', attn, vg)
        return (lambda x, *d: x.transpose(*d))(o, 0, 2, 1, 3).reshape(B, S, D) @ wo

    def _B_ref(x, mem0, Wq, Wk, Wv, Wo, seg_len):
        B, S, Dm = x.shape
        H, Dh = (Wq.shape[1], Wq.shape[2])
        M = mem0.shape[1]
        scale = Dh ** (-0.5)
        n_seg = S // seg_len
        L = M + seg_len
        idx = jnp.arange(L)
        mask = (idx[:, None] < M) | (idx[:, None] >= idx[None, :])
        mem = mem0
        outs = []
        for s in range(n_seg):
            xs = x[:, s * seg_len:(s + 1) * seg_len, :].copy()
            h = jnp.concatenate([mem, xs], axis=1)
            q = jnp.einsum('btd,dhe->bhte', h, Wq)
            k = jnp.einsum('btd,dhe->bhte', h, Wk)
            v = jnp.einsum('btd,dhe->bhte', h, Wv)
            scores = jnp.einsum('bhqe,bhke->bhqk', q, k) * scale
            scores = jnp.where(mask[None, None], scores, -1000000000.0)
            p = _softmax(scores, axis=-1)
            o = jnp.einsum('bhqk,bhke->bhqe', p, v)
            o = jnp.einsum('bhte,hed->btd', o, Wo)
            mem = o[:, :M, :].copy()
            outs.append(o[:, M:, :])
        return jnp.concatenate(outs, axis=1)
    a = _A_ref(A_x, A_wqkv, A_wo)
    b = _B_ref(B_x, B_mem0, B_Wq, B_Wk, B_Wv, B_Wo, B_seg_len)
    return jnp.concatenate([a, b], axis=-1)
```

```python
import functools

import jax
import jax.numpy as jnp
from jax import lax
from jax.experimental import pallas as pl
from jax.experimental.pallas import tpu as pltpu

F32 = jnp.float32
BF16 = jnp.bfloat16
U32 = jnp.uint32
LANES = 128
NEG = -1000000000.0

_NN = (((1,), (0,)), ((), ()))
_NT = (((1,), (1,)), ((), ()))

A_HEADS = 32
A_TAPS = 8
A_DIL = 2
A_HALO = 16
A_ROWS = 256
A_SUB = 32


def _dot(a, b, dims=_NN):
    return lax.dot_general(a, b, dims, preferred_element_type=F32)


def _b_schedule(n_pairs):
    lag_s, lag_pv, lag_o = 1, 2, 5
    seq = []
    for p in range(n_pairs):
        seq += [("q", p), ("k", p)]
        if p >= lag_s:
            seq.append(("s", p - lag_s))
        seq.append(("v", p))
        if p >= lag_pv:
            seq.append(("pv", p - lag_pv))
        if p >= lag_o:
            seq.append(("o", p - lag_o))
    n = n_pairs
    seq += [("s", n - 1), ("o", n - 5), ("pv", n - 2), ("o", n - 4), ("o", n - 3),
            ("pv", n - 1), ("o", n - 2), ("o", n - 1)]
    return seq


def _kernel(ax_hbm, wqkv_hbm, awo_hbm, bx_hbm, mem0_ref, wqt_hbm, wkt_hbm, wvt_hbm,
            bwo_hbm, out_hbm,
            ax_v, wqkv_v, awo_v, wqkv_p, awo_p, q_v, k_v, v_v, outa_v,
            bx_v, wt_v, w_v, bwo_v, outb_v,
            sem_a, sem_w, sem_b, sem_o, *, seg, n_heads):
    S, D = ax_v.shape
    NT = D // LANES
    n_blk = S // A_ROWS
    HD = bwo_hbm.shape[0]
    DH = HD // n_heads
    PW = 2 * DH
    n_pairs = n_heads // 2
    M = mem0_ref.shape[0]
    L = M + seg
    n_seg = S // seg
    CH = HD // n_blk
    wt_hbm = (wqt_hbm, wkt_hbm, wvt_hbm)

    cp_wqkv = pltpu.make_async_copy(wqkv_hbm, wqkv_v, sem_a.at[0])
    cp_awo = pltpu.make_async_copy(awo_hbm, awo_v, sem_a.at[1])
    cp_ax = pltpu.make_async_copy(ax_hbm, ax_v, sem_a.at[2])
    cp_bx = pltpu.make_async_copy(bx_hbm, bx_v, sem_b.at[0])
    cp_bwo = [pltpu.make_async_copy(bwo_hbm.at[:, pl.ds(j * LANES, LANES)], bwo_v.at[j],
                                    sem_b.at[1 + j]) for j in range(NT)]

    def cp_wt(m, c):
        r0 = pl.multiple_of(c * CH, CH)
        return pltpu.make_async_copy(wt_hbm[m].at[pl.ds(r0, CH), :],
                                     wt_v.at[m, pl.ds(r0, CH), :], sem_w.at[m, c])

    def cp_outa(i):
        r0 = pl.multiple_of(i * A_ROWS, A_ROWS)
        return pltpu.make_async_copy(outa_v.at[pl.ds(r0, A_ROWS), :],
                                     out_hbm.at[pl.ds(r0, A_ROWS), pl.ds(0, D)], sem_o.at[0])

    def cp_outb(s):
        r0 = pl.multiple_of(s * seg, seg)
        return pltpu.make_async_copy(outb_v.at[pl.ds(r0, seg), :],
                                     out_hbm.at[pl.ds(r0, seg), pl.ds(D, D)], sem_o.at[1])

    cp_wqkv.start()
    cp_awo.start()
    cp_ax.start()
    for c in range(n_blk):
        for m in range(3):
            cp_wt(m, c).start()
    for cp in cp_bwo:
        cp.start()
    cp_bx.start()

    a_dh = D // A_HEADS
    i0 = lax.broadcasted_iota(jnp.int32, (D, D), 0)
    i1 = lax.broadcasted_iota(jnp.int32, (D, D), 1)
    src = lambda c: (c & (A_HEADS - 1)) * a_dh + (c >> (A_HEADS.bit_length() - 1))
    perm = jnp.where(i0 == src(i1), 1.0, 0.0).astype(BF16)
    perm_t = jnp.where(i1 == src(i0), 1.0, 0.0).astype(BF16)
    cp_wqkv.wait()
    for j in range(3):
        t = _dot(wqkv_v[:, j * D:(j + 1) * D], perm).astype(BF16)
        wqkv_p[:, j * D:(j + 1) * D] = pltpu.bitcast(t, U32)
    cp_awo.wait()
    awo_p[...] = pltpu.bitcast(_dot(perm_t, awo_v[...]).astype(BF16), U32)
    cp_ax.wait()

    zeros = jnp.zeros((A_HALO, LANES), F32)
    for j in range(NT):
        k_v[j, 0:A_HALO, :] = zeros
        v_v[j, 0:A_HALO, :] = zeros
    a_scale = a_dh ** -0.5

    def a_block(i, carry):
        r0 = pl.multiple_of(i * A_ROWS, A_ROWS)
        x = ax_v[pl.ds(r0, A_ROWS), :]
        q_v[...] = _dot(x, pltpu.bitcast(wqkv_p[:, 0:D], BF16))
        k = _dot(x, pltpu.bitcast(wqkv_p[:, D:2 * D], BF16))
        v = _dot(x, pltpu.bitcast(wqkv_p[:, 2 * D:3 * D], BF16))
        for j in range(NT):
            k_v[j, A_HALO:A_HALO + A_ROWS, :] = k[:, j * LANES:(j + 1) * LANES]
            v_v[j, A_HALO:A_HALO + A_ROWS, :] = v[:, j * LANES:(j + 1) * LANES]

        @pl.when(i == 0)
        def _():
            for j in range(NT):
                v_v[j, 0:A_HALO, :] = jnp.broadcast_to(
                    v_v[j, A_HALO:A_HALO + 1, :], (A_HALO, LANES))

        outs = []
        for sb in range(A_ROWS // A_SUB):
            b0 = sb * A_SUB
            pos = r0 + b0 + lax.broadcasted_iota(jnp.int32, (A_SUB, LANES), 0)
            logits = []
            for w in range(A_TAPS):
                s0 = A_HALO + b0 - w * A_DIL
                t = None
                for j in range(NT):
                    pr = q_v[b0:b0 + A_SUB, j * LANES:(j + 1) * LANES] * k_v[j, s0:s0 + A_SUB, :]
                    t = pr if t is None else t + pr
                sh = LANES // 2
                while sh >= A_HEADS:
                    t = t + pltpu.roll(t, sh, 1)
                    sh //= 2
                t = t * a_scale
                if b0 < w * A_DIL:
                    t = jnp.where(pos >= w * A_DIL, t, NEG)
                logits.append(t)
            mx = functools.reduce(jnp.maximum, logits)
            es = [jnp.exp(t - mx) for t in logits]
            inv = 1.0 / functools.reduce(jnp.add, es)
            es = [e * inv for e in es]
            cols = []
            for j in range(NT):
                o = None
                for w in range(A_TAPS):
                    s0 = A_HALO + b0 - w * A_DIL
                    pr = es[w] * v_v[j, s0:s0 + A_SUB, :]
                    o = pr if o is None else o + pr
                cols.append(o)
            outs.append(jnp.concatenate(cols, axis=1).astype(BF16))
        o = jnp.concatenate(outs, axis=0)
        outa_v[pl.ds(r0, A_ROWS), :] = _dot(o, pltpu.bitcast(awo_p[...], BF16)).astype(BF16)
        for j in range(NT):
            k_v[j, 0:A_HALO, :] = k_v[j, A_ROWS:A_ROWS + A_HALO, :]
            v_v[j, 0:A_HALO, :] = v_v[j, A_ROWS:A_ROWS + A_HALO, :]
        cp_outa(i).start()

        c0 = pl.multiple_of(i * CH, CH)
        for m in range(3):
            cp_wt(m, i).wait()
        for m in range(3):
            t = wt_v[m, pl.ds(c0, CH), :].T
            w_v[m, :, pl.ds(c0, CH)] = pltpu.bitcast(t, U32)
        return carry

    lax.fori_loop(0, n_blk, a_block, 0)

    for cp in cp_bwo:
        cp.wait()
    cp_bx.wait()
    b_scale = DH ** -0.5
    schedule = _b_schedule(n_pairs)

    def b_step(s, mem):
        lane = lax.broadcasted_iota(jnp.int32, (L, PW), 1)
        lo = lane < DH
        row = lax.broadcasted_iota(jnp.int32, (L, 2 * L), 0)
        col = lax.broadcasted_iota(jnp.int32, (L, 2 * L), 1)
        in0 = col < L
        visible = (row < M) | (row >= jnp.where(in0, col, col - L))

        def split_heads(t):
            return jnp.concatenate(
                [jnp.where(lo, t, 0.0), jnp.where(lo, 0.0, t)], axis=0).astype(BF16)

        def proj(m, p):
            return _dot(h, pltpu.bitcast(w_v[m, :, p * PW:(p + 1) * PW], BF16))

        r0 = pl.multiple_of(s * seg, seg)
        h = jnp.concatenate([mem, bx_v[pl.ds(r0, seg), :].astype(F32)], axis=0)
        acc = None
        val = {}
        for op, p in schedule:
            if op == "q":
                val["q", p] = proj(0, p)
            elif op == "k":
                val["k", p] = split_heads(proj(1, p))
            elif op == "v":
                val["v", p] = split_heads(proj(2, p))
            elif op == "s":
                sc = _dot(val.pop(("q", p)), val.pop(("k", p)), _NT) * b_scale
                sc = jnp.where(visible, sc, NEG)
                m0 = jnp.max(jnp.where(in0, sc, -jnp.inf), axis=1, keepdims=True)
                m1 = jnp.max(jnp.where(in0, -jnp.inf, sc), axis=1, keepdims=True)
                e = jnp.exp(sc - jnp.where(in0, m0, m1))
                d0 = jnp.sum(jnp.where(in0, e, 0.0), axis=1, keepdims=True)
                d1 = jnp.sum(jnp.where(in0, 0.0, e), axis=1, keepdims=True)
                val["p", p] = e / jnp.where(in0, d0, d1)
            elif op == "pv":
                val["o", p] = _dot(val.pop(("p", p)), val.pop(("v", p)))
            else:
                wo = jnp.concatenate(
                    [bwo_v[j, p * PW:(p + 1) * PW, :] for j in range(NT)], axis=1)
                t = _dot(val.pop(("o", p)), wo)
                acc = t if acc is None else acc + t
        outb_v[pl.ds(r0, seg), :] = acc[M:].astype(BF16)
        cp_outb(s).start()
        return acc[:M].astype(BF16).astype(F32)

    lax.fori_loop(0, n_seg, b_step, mem0_ref[...].astype(F32))

    pltpu.make_async_copy(outa_v, out_hbm.at[:, pl.ds(0, D)], sem_o.at[0]).wait()
    pltpu.make_async_copy(outb_v, out_hbm.at[:, pl.ds(D, D)], sem_o.at[1]).wait()


@functools.partial(jax.jit, static_argnames=("B_seg_len",))
def pallas_concat_heads__sliding_local_dilated__memory_aug_recurrent_mem_tr__prompt_kernel(
    A_x: jax.Array,
    A_wqkv: jax.Array,
    A_wo: jax.Array,
    B_x: jax.Array,
    B_mem0: jax.Array,
    B_Wq: jax.Array,
    B_Wk: jax.Array,
    B_Wv: jax.Array,
    B_Wo: jax.Array,
    B_seg_len: int,
):
    B, S, D = A_x.shape
    _, H, DH = B_Wq.shape
    M = B_mem0.shape[1]
    HD = H * DH
    NT = D // LANES
    n_blk = S // A_ROWS
    assert B == 1 and B_x.shape == A_x.shape and A_x.dtype == BF16

    wt = lambda w: w.transpose(1, 2, 0).reshape(HD, D)
    hbm = pl.BlockSpec(memory_space=pl.ANY)
    out = pl.pallas_call(
        functools.partial(_kernel, seg=int(B_seg_len), n_heads=H),
        out_shape=jax.ShapeDtypeStruct((S, 2 * D), BF16),
        in_specs=[hbm, hbm, hbm, hbm, pl.BlockSpec(memory_space=pltpu.VMEM),
                  hbm, hbm, hbm, hbm],
        out_specs=hbm,
        scratch_shapes=[
            pltpu.VMEM((S, D), BF16),
            pltpu.VMEM((D, 3 * D), BF16),
            pltpu.VMEM((D, D), BF16),
            pltpu.VMEM((D // 2, 3 * D), U32),
            pltpu.VMEM((D // 2, D), U32),
            pltpu.VMEM((A_ROWS, D), F32),
            pltpu.VMEM((NT, A_HALO + A_ROWS, LANES), F32),
            pltpu.VMEM((NT, A_HALO + A_ROWS, LANES), F32),
            pltpu.VMEM((S, D), BF16),
            pltpu.VMEM((S, D), BF16),
            pltpu.VMEM((3, HD, D), BF16),
            pltpu.VMEM((3, D // 2, HD), U32),
            pltpu.VMEM((NT, HD, LANES), BF16),
            pltpu.VMEM((S, D), BF16),
            pltpu.SemaphoreType.DMA((3,)),
            pltpu.SemaphoreType.DMA((3, n_blk)),
            pltpu.SemaphoreType.DMA((1 + NT,)),
            pltpu.SemaphoreType.DMA((2,)),
        ],
        compiler_params=pltpu.CompilerParams(vmem_limit_bytes=110 << 20),
    )(A_x.reshape(S, D), A_wqkv, A_wo, B_x.reshape(S, D), B_mem0.reshape(M, D),
      wt(B_Wq), wt(B_Wk), wt(B_Wv), B_Wo.reshape(HD, D))
    return out.reshape(B, S, 2 * D)
```

```python
import functools

import jax
import jax.numpy as jnp
from jax import lax
from jax.experimental import pallas as pl
from jax.experimental.pallas import tpu as pltpu

F32 = jnp.float32
BF16 = jnp.bfloat16
U32 = jnp.uint32
LANES = 128
NEG = -1000000000.0

_NN = (((1,), (0,)), ((), ()))
_NT = (((1,), (1,)), ((), ()))

A_HEADS = 32
A_TAPS = 8
A_DIL = 2
A_HALO = 16
A_ROWS = 128
A_SUB = 32
W_AHEAD = 3


def _dot(a, b, dims=_NN):
    return lax.dot_general(a, b, dims, preferred_element_type=F32)


def _b_schedule(n_pairs):
    lag_s, lag_pv, lag_o = 1, 2, 5
    seq = []
    for p in range(n_pairs):
        seq += [("q", p), ("k", p)]
        if p >= lag_s:
            seq.append(("s", p - lag_s))
        seq.append(("v", p))
        if p >= lag_pv:
            seq.append(("pv", p - lag_pv))
        if p >= lag_o:
            seq.append(("o", p - lag_o))
    n = n_pairs
    seq += [("s", n - 1), ("o", n - 5), ("pv", n - 2), ("o", n - 4), ("o", n - 3),
            ("pv", n - 1), ("o", n - 2), ("o", n - 1)]
    return seq


def _kernel(ax_hbm, wqkv_hbm, awo_hbm, bx_hbm, mem0_ref, wqt_hbm, wkt_hbm, wvt_hbm,
            bwo_hbm, out_hbm,
            ax_v, wqkv_v, awo_v, wqkv_p, awo_p, q0_v, k0_v, v0_v, q1_v, k1_v, v1_v, outa_v,
            bx_v, wt_v, w_v, bwo_v, outb_v,
            sem_a, sem_w, sem_o, *, seg, n_heads):
    S, D = ax_v.shape
    NT = D // LANES
    n_blk = S // A_ROWS
    n_it = n_blk // 2
    HD = bwo_hbm.shape[0]
    DH = HD // n_heads
    PW = 2 * DH
    n_pairs = n_heads // 2
    M = mem0_ref.shape[0]
    L = M + seg
    n_seg = S // seg
    CH = HD // n_it
    w_hbm = (wqt_hbm, wkt_hbm, wvt_hbm)

    head = 2 * seg
    cp_wqkv = pltpu.make_async_copy(wqkv_hbm, wqkv_v, sem_a.at[0])
    cp_awo = pltpu.make_async_copy(awo_hbm, awo_v, sem_a.at[1])
    cp_ax = pltpu.make_async_copy(ax_hbm, ax_v, sem_a.at[2])
    cp_bx0 = pltpu.make_async_copy(bx_hbm.at[pl.ds(0, head), :], bx_v.at[pl.ds(0, head), :],
                                   sem_a.at[3])
    cp_bx1 = pltpu.make_async_copy(bx_hbm.at[pl.ds(head, S - head), :],
                                   bx_v.at[pl.ds(head, S - head), :], sem_a.at[4])
    cp_outa = pltpu.make_async_copy(outa_v, out_hbm.at[:, pl.ds(0, D)], sem_o.at[0])

    def cp_wt(m, c):
        r0 = pl.multiple_of(c * CH, CH)
        return pltpu.make_async_copy(w_hbm[m].at[pl.ds(r0, CH), :],
                                     wt_v.at[m, pl.ds(r0, CH), :], sem_w.at[m, c])

    def cp_bwo(c):
        r0 = pl.multiple_of(c * CH, CH)
        return pltpu.make_async_copy(bwo_hbm.at[pl.ds(r0, CH), :],
                                     bwo_v.at[pl.ds(r0, CH), :], sem_w.at[3, c])

    def cp_outb(s):
        r0 = pl.multiple_of(s * seg, seg)
        return pltpu.make_async_copy(outb_v.at[pl.ds(r0, seg), :],
                                     out_hbm.at[pl.ds(r0, seg), pl.ds(D, D)], sem_o.at[1])

    cp_wqkv.start()

    a_dh = D // A_HEADS
    i0 = lax.broadcasted_iota(jnp.int32, (D, D), 0)
    i1 = lax.broadcasted_iota(jnp.int32, (D, D), 1)
    src = lambda c: (c & (A_HEADS - 1)) * a_dh + (c >> (A_HEADS.bit_length() - 1))
    perm = jnp.where(i0 == src(i1), 1.0, 0.0).astype(BF16)
    perm_t = jnp.where(i1 == src(i0), 1.0, 0.0).astype(BF16)
    zeros = jnp.zeros((A_HALO, LANES), F32)
    for j in range(NT):
        k1_v[j, A_ROWS:, :] = zeros
    cp_awo.start()
    cp_ax.start()
    cp_wqkv.wait()
    for c in range(W_AHEAD):
        for m in range(3):
            cp_wt(m, c).start()
    cp_bx0.start()
    for j in range(3):
        t = _dot(wqkv_v[:, j * D:(j + 1) * D], perm).astype(BF16)
        wqkv_p[:, j * D:(j + 1) * D] = pltpu.bitcast(t, U32)
    cp_awo.wait()
    awo_p[...] = pltpu.bitcast(_dot(perm_t, awo_v[...]).astype(BF16), U32)
    cp_ax.wait()
    a_scale = a_dh ** -0.5

    def a_project(n, buf):
        q_v, k_v, v_v = buf
        x = ax_v[pl.ds(pl.multiple_of(n * A_ROWS, A_ROWS), A_ROWS), :]
        q_v[...] = _dot(x, pltpu.bitcast(wqkv_p[:, 0:D], BF16))
        k = _dot(x, pltpu.bitcast(wqkv_p[:, D:2 * D], BF16))
        v = _dot(x, pltpu.bitcast(wqkv_p[:, 2 * D:3 * D], BF16))
        for j in range(NT):
            k_v[j, A_HALO:, :] = k[:, j * LANES:(j + 1) * LANES]
            v_v[j, A_HALO:, :] = v[:, j * LANES:(j + 1) * LANES]

    def a_attend(n, buf):
        q_v, k_v, v_v = buf
        outs = []
        for b0 in range(0, A_ROWS, A_SUB):
            pos = n * A_ROWS + b0 + lax.broadcasted_iota(jnp.int32, (A_SUB, LANES), 0)
            logits = []
            for w in range(A_TAPS):
                s0 = A_HALO + b0 - w * A_DIL
                t = None
                for j in range(NT):
                    pr = q_v[b0:b0 + A_SUB, j * LANES:(j + 1) * LANES] * k_v[j, s0:s0 + A_SUB, :]
                    t = pr if t is None else t + pr
                sh = LANES // 2
                while sh >= A_HEADS:
                    t = t + pltpu.roll(t, sh, 1)
                    sh //= 2
                t = t * a_scale
                if b0 < w * A_DIL:
                    t = jnp.where(pos >= w * A_DIL, t, NEG)
                logits.append(t)
            mx = functools.reduce(jnp.maximum, logits)
            es = [jnp.exp(t - mx) for t in logits]
            inv = 1.0 / functools.reduce(jnp.add, es)
            es = [e * inv for e in es]
            cols = []
            for j in range(NT):
                o = None
                for w in range(A_TAPS):
                    s0 = A_HALO + b0 - w * A_DIL
                    pr = es[w] * v_v[j, s0:s0 + A_SUB, :]
                    o = pr if o is None else o + pr
                cols.append(o)
            outs.append(jnp.concatenate(cols, axis=1).astype(BF16))
        return jnp.concatenate(outs, axis=0)

    def a_half(n, cur, nxt, c0):
        for dst, prev in zip(cur[1:], nxt[1:]):
            for j in range(NT):
                dst[j, 0:A_HALO, :] = prev[j, A_ROWS:, :]
        a_project(jnp.minimum(n + 1, n_blk - 1), nxt)
        o = a_attend(n, cur)
        outa_v[pl.ds(pl.multiple_of(n * A_ROWS, A_ROWS), A_ROWS), :] = _dot(
            o, pltpu.bitcast(awo_p[...], BF16)).astype(BF16)
        c0 = pl.multiple_of(c0, CH // 2)
        for m in range(3):
            w_v[m, :, pl.ds(c0, CH // 2)] = pltpu.bitcast(wt_v[m, pl.ds(c0, CH // 2), :].T, U32)

    buf0, buf1 = (q0_v, k0_v, v0_v), (q1_v, k1_v, v1_v)
    a_project(0, buf0)
    for j in range(NT):
        v1_v[j, A_ROWS:, :] = jnp.broadcast_to(v0_v[j, A_HALO:A_HALO + 1, :], (A_HALO, LANES))

    def a_iter(i, carry):
        @pl.when(i + W_AHEAD < n_it)
        def _():
            for m in range(3):
                cp_wt(m, i + W_AHEAD).start()
        cp_bwo(i).start()
        for m in range(3):
            cp_wt(m, i).wait()
        a_half(2 * i, buf0, buf1, i * CH)
        a_half(2 * i + 1, buf1, buf0, i * CH + CH // 2)
        return carry

    lax.fori_loop(0, n_it, a_iter, 0)

    for c in range(n_it):
        cp_bwo(c).wait()
    cp_bx0.wait()
    cp_bx1.start()
    cp_outa.start()
    b_scale = DH ** -0.5
    schedule = _b_schedule(n_pairs)

    def b_step(s, mem):
        @pl.when(s == head // seg)
        def _():
            cp_bx1.wait()

        lane = lax.broadcasted_iota(jnp.int32, (L, PW), 1)
        lo = lane < DH
        row = lax.broadcasted_iota(jnp.int32, (L, 2 * L), 0)
        col = lax.broadcasted_iota(jnp.int32, (L, 2 * L), 1)
        in0 = col < L
        visible = (row < M) | (row >= jnp.where(in0, col, col - L))

        def split_heads(t):
            return jnp.concatenate(
                [jnp.where(lo, t, 0.0), jnp.where(lo, 0.0, t)], axis=0).astype(BF16)

        def proj(m, p):
            return _dot(h, pltpu.bitcast(w_v[m, :, p * PW:(p + 1) * PW], BF16))

        r0 = pl.multiple_of(s * seg, seg)
        h = jnp.concatenate([mem, bx_v[pl.ds(r0, seg), :].astype(F32)], axis=0)
        acc = None
        val = {}
        for op, p in schedule:
            if op == "q":
                val["q", p] = proj(0, p)
            elif op == "k":
                val["k", p] = split_heads(proj(1, p))
            elif op == "v":
                val["v", p] = split_heads(proj(2, p))
            elif op == "s":
                sc = _dot(val.pop(("q", p)), val.pop(("k", p)), _NT) * b_scale
                sc = jnp.where(visible, sc, NEG)
                m0 = jnp.max(jnp.where(in0, sc, -jnp.inf), axis=1, keepdims=True)
                m1 = jnp.max(jnp.where(in0, -jnp.inf, sc), axis=1, keepdims=True)
                e = jnp.exp(sc - jnp.where(in0, m0, m1))
                d0 = jnp.sum(jnp.where(in0, e, 0.0), axis=1, keepdims=True)
                d1 = jnp.sum(jnp.where(in0, 0.0, e), axis=1, keepdims=True)
                val["p", p] = e / jnp.where(in0, d0, d1)
            elif op == "pv":
                val["o", p] = _dot(val.pop(("p", p)), val.pop(("v", p)))
            else:
                t = _dot(val.pop(("o", p)), bwo_v[p * PW:(p + 1) * PW, :])
                acc = t if acc is None else acc + t
        outb_v[pl.ds(r0, seg), :] = acc[M:].astype(BF16)
        cp_outb(s).start()
        return acc[:M].astype(BF16).astype(F32)

    lax.fori_loop(0, n_seg, b_step, mem0_ref[...].astype(F32))

    cp_outa.wait()
    pltpu.make_async_copy(outb_v, out_hbm.at[:, pl.ds(D, D)], sem_o.at[1]).wait()


@functools.partial(jax.jit, static_argnames=("B_seg_len",))
def pallas_concat_heads__sliding_local_dilated__memory_aug_recurrent_mem_tr__prompt_kernel(
    A_x: jax.Array,
    A_wqkv: jax.Array,
    A_wo: jax.Array,
    B_x: jax.Array,
    B_mem0: jax.Array,
    B_Wq: jax.Array,
    B_Wk: jax.Array,
    B_Wv: jax.Array,
    B_Wo: jax.Array,
    B_seg_len: int,
):
    B, S, D = A_x.shape
    _, H, DH = B_Wq.shape
    M = B_mem0.shape[1]
    HD = H * DH
    NT = D // LANES
    n_blk = S // A_ROWS
    assert B == 1 and B_x.shape == A_x.shape and A_x.dtype == BF16

    wt = lambda w: w.transpose(1, 2, 0).reshape(HD, D)
    hbm = pl.BlockSpec(memory_space=pl.ANY)
    out = pl.pallas_call(
        functools.partial(_kernel, seg=int(B_seg_len), n_heads=H),
        out_shape=jax.ShapeDtypeStruct((S, 2 * D), BF16),
        in_specs=[hbm, hbm, hbm, hbm, pl.BlockSpec(memory_space=pltpu.VMEM),
                  hbm, hbm, hbm, hbm],
        out_specs=hbm,
        scratch_shapes=[
            pltpu.VMEM((S, D), BF16),
            pltpu.VMEM((D, 3 * D), BF16),
            pltpu.VMEM((D, D), BF16),
            pltpu.VMEM((D // 2, 3 * D), U32),
            pltpu.VMEM((D // 2, D), U32),
            *([pltpu.VMEM((A_ROWS, D), F32),
               pltpu.VMEM((NT, A_HALO + A_ROWS, LANES), F32),
               pltpu.VMEM((NT, A_HALO + A_ROWS, LANES), F32)] * 2),
            pltpu.VMEM((S, D), BF16),
            pltpu.VMEM((S, D), BF16),
            pltpu.VMEM((3, HD, D), BF16),
            pltpu.VMEM((3, D // 2, HD), U32),
            pltpu.VMEM((HD, D), BF16),
            pltpu.VMEM((S, D), BF16),
            pltpu.SemaphoreType.DMA((5,)),
            pltpu.SemaphoreType.DMA((4, n_blk // 2)),
            pltpu.SemaphoreType.DMA((2,)),
        ],
        compiler_params=pltpu.CompilerParams(vmem_limit_bytes=110 << 20),
    )(A_x.reshape(S, D), A_wqkv, A_wo, B_x.reshape(S, D), B_mem0.reshape(M, D),
      wt(B_Wq), wt(B_Wk), wt(B_Wv), B_Wo.reshape(HD, D))
    return out.reshape(B, S, 2 * D)
```

```python
import functools

import jax
import jax.numpy as jnp
from jax import lax
from jax.experimental import pallas as pl
from jax.experimental.pallas import tpu as pltpu

F32 = jnp.float32
BF16 = jnp.bfloat16
U32 = jnp.uint32
LANES = 128
NEG = -1000000000.0

_NN = (((1,), (0,)), ((), ()))
_NT = (((1,), (1,)), ((), ()))

A_HEADS = 32
A_TAPS = 8
A_DIL = 2
A_HALO = 16
A_ROWS = 128
A_SUB = 32
BWO_START = (5, 5, 6, 6, 6, 7, 7, 7)


def _dot(a, b, dims=_NN):
    return lax.dot_general(a, b, dims, preferred_element_type=F32)


def _b_schedule(n_pairs):
    lag_s, lag_pv, lag_o = 1, 2, 5
    seq = []
    for p in range(n_pairs):
        seq += [("q", p), ("k", p)]
        if p >= lag_s:
            seq.append(("s", p - lag_s))
        seq.append(("v", p))
        if p >= lag_pv:
            seq.append(("pv", p - lag_pv))
        if p >= lag_o:
            seq.append(("o", p - lag_o))
    n = n_pairs
    seq += [("s", n - 1), ("o", n - 5), ("pv", n - 2), ("o", n - 4), ("o", n - 3),
            ("pv", n - 1), ("o", n - 2), ("o", n - 1)]
    return seq


def _kernel(ax_hbm, wqkv_hbm, awo_hbm, bx_hbm, mem0_ref, wqt_hbm, wkt_hbm, wvt_hbm,
            bwo_hbm, out_hbm,
            ax_v, wqkv_v, awo_v, perm_v, wqkv_p, awo_p, q0_v, k0_v, v0_v, q1_v, k1_v, v1_v, outa_v,
            bx_v, wt_v, w_v, bwo_v, outb_v,
            sem_a, sem_w, sem_o, *, seg, n_heads):
    S, D = ax_v.shape
    NT = D // LANES
    n_blk = S // A_ROWS
    n_it = n_blk // 2
    HD = bwo_hbm.shape[0]
    DH = HD // n_heads
    PW = 2 * DH
    n_pairs = n_heads // 2
    M = mem0_ref.shape[0]
    L = M + seg
    n_seg = S // seg
    CH = HD // n_it
    w_hbm = (wqt_hbm, wkt_hbm, wvt_hbm)

    head = 2 * seg
    cp_wqkv = pltpu.make_async_copy(wqkv_hbm, wqkv_v, sem_a.at[0])
    cp_awo = pltpu.make_async_copy(awo_hbm, awo_v, sem_a.at[1])
    cp_bx0 = pltpu.make_async_copy(bx_hbm.at[pl.ds(0, head), :], bx_v.at[pl.ds(0, head), :],
                                   sem_a.at[2])
    cp_bx1 = pltpu.make_async_copy(bx_hbm.at[pl.ds(head, S - head), :],
                                   bx_v.at[pl.ds(head, S - head), :], sem_a.at[3])
    cp_outa = pltpu.make_async_copy(outa_v, out_hbm.at[:, pl.ds(0, D)], sem_o.at[0])

    def rows_copy(src, dst, rows, c, sem):
        r0 = pl.multiple_of(c * rows, rows)
        return pltpu.make_async_copy(src.at[pl.ds(r0, rows), :], dst.at[pl.ds(r0, rows), :], sem)

    cp_wt = lambda m, c: rows_copy(w_hbm[m], wt_v.at[m], CH, c, sem_w.at[m, c])
    cp_bwo = lambda c: rows_copy(bwo_hbm, bwo_v, CH, c, sem_w.at[3, c])
    cp_ax = lambda c: rows_copy(ax_hbm, ax_v, 2 * A_ROWS, c, sem_w.at[4, c])

    def cp_outb(s):
        r0 = pl.multiple_of(s * seg, seg)
        return pltpu.make_async_copy(outb_v.at[pl.ds(r0, seg), :],
                                     out_hbm.at[pl.ds(r0, seg), pl.ds(D, D)], sem_o.at[1])

    def start_wt(c):
        for m in range(3):
            cp_wt(m, c).start()

    def wait_wt(c):
        for m in range(3):
            cp_wt(m, c).wait()

    def transpose_wt(c, half):
        c0 = pl.multiple_of(c * CH + half * (CH // 2), CH // 2)
        for m in range(3):
            w_v[m, :, pl.ds(c0, CH // 2)] = pltpu.bitcast(wt_v[m, pl.ds(c0, CH // 2), :].T, U32)

    a_dh = D // A_HEADS
    a_scale = a_dh ** -0.5

    def permute_rows(j, rows):
        rows = rows.astype(F32)
        for t in range(NT):
            perm_v[j, t] = rows[:, t * LANES:(t + 1) * LANES]
        rows = [jnp.concatenate([perm_v[j, t, pl.ds(d, A_HEADS, stride=a_dh), :]
                                 for t in range(NT)], axis=1) for d in range(a_dh)]
        return pltpu.bitcast(jnp.concatenate(rows, axis=0).astype(BF16), U32)

    def a_project(n, buf):
        q_v, k_v, v_v = buf
        x = ax_v[pl.ds(pl.multiple_of(n * A_ROWS, A_ROWS), A_ROWS), :]
        q_v[...] = _dot(x, pltpu.bitcast(wqkv_p[0], BF16), _NT)
        k = _dot(x, pltpu.bitcast(wqkv_p[1], BF16), _NT)
        v = _dot(x, pltpu.bitcast(wqkv_p[2], BF16), _NT)
        for j in range(NT):
            k_v[j, A_HALO:, :] = k[:, j * LANES:(j + 1) * LANES]
            v_v[j, A_HALO:, :] = v[:, j * LANES:(j + 1) * LANES]

    def a_halo(cur, prev):
        for dst, src in zip(cur[1:], prev[1:]):
            for j in range(NT):
                dst[j, 0:A_HALO, :] = src[j, A_ROWS:, :]

    def a_attend(buf, first=False):
        q_v, k_v, v_v = buf
        outs = []
        for b0 in range(0, A_ROWS, A_SUB):
            logits = []
            for w in range(A_TAPS):
                s0 = A_HALO + b0 - w * A_DIL
                t = None
                for j in range(NT):
                    pr = q_v[b0:b0 + A_SUB, j * LANES:(j + 1) * LANES] * k_v[j, s0:s0 + A_SUB, :]
                    t = pr if t is None else t + pr
                sh = LANES // 2
                while sh >= A_HEADS:
                    t = t + pltpu.roll(t, sh, 1)
                    sh //= 2
                t = t * a_scale
                if first and b0 < w * A_DIL:
                    pos = b0 + lax.broadcasted_iota(jnp.int32, (A_SUB, LANES), 0)
                    t = jnp.where(pos >= w * A_DIL, t, NEG)
                logits.append(t)
            mx = functools.reduce(jnp.maximum, logits)
            es = [jnp.exp(t - mx) for t in logits]
            inv = 1.0 / functools.reduce(jnp.add, es)
            es = [e * inv for e in es]
            cols = []
            for j in range(NT):
                o = None
                for w in range(A_TAPS):
                    s0 = A_HALO + b0 - w * A_DIL
                    pr = es[w] * v_v[j, s0:s0 + A_SUB, :]
                    o = pr if o is None else o + pr
                cols.append(o)
            outs.append(jnp.concatenate(cols, axis=1).astype(BF16))
        return jnp.concatenate(outs, axis=0)

    def a_output(n, o):
        outa_v[pl.ds(pl.multiple_of(n * A_ROWS, A_ROWS), A_ROWS), :] = _dot(
            o, pltpu.bitcast(awo_p[...], BF16)).astype(BF16)

    buf0, buf1 = (q0_v, k0_v, v0_v), (q1_v, k1_v, v1_v)
    cp_wqkv.start()
    cp_ax(0).start()
    cp_awo.start()
    cp_wqkv.wait()
    start_wt(0)
    cp_ax(1).start()
    cp_bx0.start()
    for j in range(3):
        wqkv_p[j] = permute_rows(j, wqkv_v[:, j * D:(j + 1) * D].T)
    cp_awo.wait()
    awo_p[...] = permute_rows(3, awo_v[...])
    cp_ax(0).wait()
    a_project(0, buf0)
    start_wt(1)
    cp_ax(2).start()
    for t_v in buf0[1:]:
        for j in range(NT):
            t_v[j, 0:A_HALO, :] = jnp.broadcast_to(t_v[j, A_HALO:A_HALO + 1, :], (A_HALO, LANES))
    a_project(1, buf1)
    a_output(0, a_attend(buf0, first=True))

    def a_iter(i, carry):
        @pl.when(i + 2 < n_it)
        def _():
            start_wt(i + 2)

        @pl.when(i + 3 < n_it)
        def _():
            cp_ax(i + 3).start()

        for c, at in enumerate(BWO_START):
            if at < n_it - 1:
                pl.when(i == at)(cp_bwo(c).start)
        cp_ax(i + 1).wait()
        wait_wt(i)
        for half, (cur, nxt) in enumerate(((buf1, buf0), (buf0, buf1))):
            n = 2 * i + 1 + half
            a_halo(cur, nxt)
            a_project(n + 1, nxt)
            a_output(n, a_attend(cur))
            transpose_wt(i, half)
        return carry

    lax.fori_loop(0, n_it - 1, a_iter, 0)

    b_scale = DH ** -0.5
    schedule = _b_schedule(n_pairs)

    def b_step(s, mem, before=None):
        lane = lax.broadcasted_iota(jnp.int32, (L, PW), 1)
        lo = lane < DH
        row = lax.broadcasted_iota(jnp.int32, (L, 2 * L), 0)
        col = lax.broadcasted_iota(jnp.int32, (L, 2 * L), 1)
        in0 = col < L
        visible = (row < M) | (row >= jnp.where(in0, col, col - L))

        def split_heads(t):
            return jnp.concatenate(
                [jnp.where(lo, t, 0.0), jnp.where(lo, 0.0, t)], axis=0).astype(BF16)

        def proj(m, p):
            return _dot(h, pltpu.bitcast(w_v[m, :, p * PW:(p + 1) * PW], BF16))

        r0 = pl.multiple_of(s * seg, seg)
        h = jnp.concatenate([mem, bx_v[pl.ds(r0, seg), :].astype(F32)], axis=0)
        acc = None
        val = {}
        for op, p in schedule:
            if before is not None:
                before(op, p)
            if op == "q":
                val["q", p] = proj(0, p)
            elif op == "k":
                val["k", p] = split_heads(proj(1, p))
            elif op == "v":
                val["v", p] = split_heads(proj(2, p))
            elif op == "s":
                sc = _dot(val.pop(("q", p)), val.pop(("k", p)), _NT) * b_scale
                sc = jnp.where(visible, sc, NEG)
                m0 = jnp.max(jnp.where(in0, sc, -jnp.inf), axis=1, keepdims=True)
                m1 = jnp.max(jnp.where(in0, -jnp.inf, sc), axis=1, keepdims=True)
                e = jnp.exp(sc - jnp.where(in0, m0, m1))
                d0 = jnp.sum(jnp.where(in0, e, 0.0), axis=1, keepdims=True)
                d1 = jnp.sum(jnp.where(in0, 0.0, e), axis=1, keepdims=True)
                val["p", p] = e / jnp.where(in0, d0, d1)
            elif op == "pv":
                val["o", p] = _dot(val.pop(("p", p)), val.pop(("v", p)))
            else:
                t = _dot(val.pop(("o", p)), bwo_v[p * PW:(p + 1) * PW, :])
                acc = t if acc is None else acc + t
        outb_v[pl.ds(r0, seg), :] = acc[M:].astype(BF16)
        cp_outb(s).start()
        return acc[:M].astype(BF16).astype(F32)

    for c, at in enumerate(BWO_START):
        if at == n_it - 1:
            cp_bwo(c).start()
    wait_wt(n_it - 1)
    cp_bx0.wait()
    a_halo(buf1, buf0)
    o_last = a_attend(buf1)
    transpose_wt(n_it - 1, 0)
    transpose_wt(n_it - 1, 1)

    def first_step_hook(op, p):
        if (op, p) == ("q", 4):
            a_output(n_blk - 1, o_last)
        if op == "o" and p * PW % CH == 0:
            cp_bwo(p * PW // CH).wait()

    mem = b_step(0, mem0_ref[...].astype(F32), first_step_hook)
    cp_bx1.start()
    cp_outa.start()

    def b_iter(s, mem):
        pl.when(s == head // seg)(cp_bx1.wait)
        return b_step(s, mem)

    lax.fori_loop(1, n_seg, b_iter, mem)

    cp_outa.wait()
    pltpu.make_async_copy(outb_v, out_hbm.at[:, pl.ds(D, D)], sem_o.at[1]).wait()


@functools.partial(jax.jit, static_argnames=("B_seg_len",))
def pallas_concat_heads__sliding_local_dilated__memory_aug_recurrent_mem_tr__prompt_kernel(
    A_x: jax.Array,
    A_wqkv: jax.Array,
    A_wo: jax.Array,
    B_x: jax.Array,
    B_mem0: jax.Array,
    B_Wq: jax.Array,
    B_Wk: jax.Array,
    B_Wv: jax.Array,
    B_Wo: jax.Array,
    B_seg_len: int,
):
    B, S, D = A_x.shape
    _, H, DH = B_Wq.shape
    M = B_mem0.shape[1]
    HD = H * DH
    NT = D // LANES
    n_blk = S // A_ROWS
    assert B == 1 and B_x.shape == A_x.shape and A_x.dtype == BF16

    wt = lambda w: w.transpose(1, 2, 0).reshape(HD, D)
    hbm = pl.BlockSpec(memory_space=pl.ANY)
    out = pl.pallas_call(
        functools.partial(_kernel, seg=int(B_seg_len), n_heads=H),
        out_shape=jax.ShapeDtypeStruct((S, 2 * D), BF16),
        in_specs=[hbm, hbm, hbm, hbm, pl.BlockSpec(memory_space=pltpu.VMEM),
                  hbm, hbm, hbm, hbm],
        out_specs=hbm,
        scratch_shapes=[
            pltpu.VMEM((S, D), BF16),
            pltpu.VMEM((D, 3 * D), BF16),
            pltpu.VMEM((D, D), BF16),
            pltpu.VMEM((4, NT, D, LANES), F32),
            pltpu.VMEM((3, D // 2, D), U32),
            pltpu.VMEM((D // 2, D), U32),
            *([pltpu.VMEM((A_ROWS, D), F32),
               pltpu.VMEM((NT, A_HALO + A_ROWS, LANES), F32),
               pltpu.VMEM((NT, A_HALO + A_ROWS, LANES), F32)] * 2),
            pltpu.VMEM((S, D), BF16),
            pltpu.VMEM((S, D), BF16),
            pltpu.VMEM((3, HD, D), BF16),
            pltpu.VMEM((3, D // 2, HD), U32),
            pltpu.VMEM((HD, D), BF16),
            pltpu.VMEM((S, D), BF16),
            pltpu.SemaphoreType.DMA((4,)),
            pltpu.SemaphoreType.DMA((5, n_blk // 2)),
            pltpu.SemaphoreType.DMA((2,)),
        ],
        compiler_params=pltpu.CompilerParams(vmem_limit_bytes=110 << 20),
    )(A_x.reshape(S, D), A_wqkv, A_wo, B_x.reshape(S, D), B_mem0.reshape(M, D),
      wt(B_Wq), wt(B_Wk), wt(B_Wv), B_Wo.reshape(HD, D))
    return out.reshape(B, S, 2 * D)
```

```python
import functools

import jax
import jax.numpy as jnp
from jax import lax
from jax.experimental import pallas as pl
from jax.experimental.pallas import tpu as pltpu

F32 = jnp.float32
BF16 = jnp.bfloat16
U32 = jnp.uint32
LANES = 128
NEG = -1000000000.0

_NN = (((1,), (0,)), ((), ()))
_NT = (((1,), (1,)), ((), ()))

A_HEADS = 32
A_TAPS = 8
A_DIL = 2
A_HALO = 16
A_ROWS = 256
A_SUB = 16
W_AHEAD = 3
BWO_START = (5, 6)


def _dot(a, b, dims=_NN):
    return lax.dot_general(a, b, dims, preferred_element_type=F32)


def _interleave(*streams):
    order = [((i + 0.5) / len(st), k, i) for k, st in enumerate(streams) for i in range(len(st))]
    for _, k, i in sorted(order):
        streams[k][i]()


def _b_schedule(n_pairs):
    lag_s, lag_pv, lag_o = 1, 2, 5
    seq = []
    for p in range(n_pairs):
        seq += [("q", p), ("k", p)]
        if p >= lag_s:
            seq.append(("s", p - lag_s))
        seq.append(("v", p))
        if p >= lag_pv:
            seq.append(("pv", p - lag_pv))
        if p >= lag_o:
            seq.append(("o", p - lag_o))
    n = n_pairs
    seq += [("s", n - 1), ("o", n - 5), ("pv", n - 2), ("o", n - 4), ("o", n - 3),
            ("pv", n - 1), ("o", n - 2), ("o", n - 1)]
    return seq


def _kernel(ax_hbm, wqkv_hbm, awo_hbm, bx_hbm, mem0_ref, wqt_hbm, wkt_hbm, wvt_hbm,
            bwo_hbm, out_hbm,
            ax_v, wqkv_v, awo_v, perm_v, wqkv_p, awo_p, qkvo_v, outa_v,
            bx_v, wt_v, w_v, bwo_v, outb_v,
            sem_a, sem_w, sem_o, *, seg, n_heads):
    S, D = ax_v.shape
    NT = D // LANES
    n_blk = S // A_ROWS
    HD = bwo_hbm.shape[0]
    DH = HD // n_heads
    PW = 2 * DH
    n_pairs = n_heads // 2
    M = mem0_ref.shape[0]
    L = M + seg
    n_seg = S // seg
    CH = HD // n_blk
    w_hbm = (wqt_hbm, wkt_hbm, wvt_hbm)

    head = 2 * seg
    cp_wqkv = pltpu.make_async_copy(wqkv_hbm, wqkv_v, sem_a.at[0])
    cp_awo = pltpu.make_async_copy(awo_hbm, awo_v, sem_a.at[1])
    cp_bx0 = pltpu.make_async_copy(bx_hbm.at[pl.ds(0, head), :], bx_v.at[pl.ds(0, head), :],
                                   sem_a.at[2])
    cp_bx1 = pltpu.make_async_copy(bx_hbm.at[pl.ds(head, S - head), :],
                                   bx_v.at[pl.ds(head, S - head), :], sem_a.at[3])
    cp_outa = pltpu.make_async_copy(outa_v, out_hbm.at[:, pl.ds(0, D)], sem_o.at[0])

    def rows_copy(src, dst, rows, c, sem):
        r0 = pl.multiple_of(c * rows, rows)
        return pltpu.make_async_copy(src.at[pl.ds(r0, rows), :], dst.at[pl.ds(r0, rows), :], sem)

    cp_wt = lambda m, c: rows_copy(w_hbm[m], wt_v.at[m], CH, c, sem_w.at[m, c])
    cp_bwo = lambda c: rows_copy(bwo_hbm, bwo_v, HD // len(BWO_START), c, sem_a.at[4 + c])
    cp_ax = lambda c: rows_copy(ax_hbm, ax_v, A_ROWS, c, sem_w.at[3, c])

    def cp_outb(s):
        r0 = pl.multiple_of(s * seg, seg)
        return pltpu.make_async_copy(outb_v.at[pl.ds(r0, seg), :],
                                     out_hbm.at[pl.ds(r0, seg), pl.ds(D, D)], sem_o.at[1])

    def start_wt(c):
        for m in range(3):
            cp_wt(m, c).start()

    def wait_wt(c):
        for m in range(3):
            cp_wt(m, c).wait()

    def transpose_wt(c):
        def piece(m, t):
            c0 = pl.multiple_of(c * CH + t * LANES, LANES)
            w_v[m, :, pl.ds(c0, LANES)] = pltpu.bitcast(wt_v[m, pl.ds(c0, LANES), :].T, U32)
        return [functools.partial(piece, m, t) for t in range(CH // LANES) for m in range(3)]

    a_dh = D // A_HEADS
    a_scale = a_dh ** -0.5

    def permute_rows(j, rows):
        rows = rows.astype(F32)
        for t in range(NT):
            perm_v[j, t] = rows[:, t * LANES:(t + 1) * LANES]
        rows = [jnp.concatenate([perm_v[j, t, pl.ds(d, A_HEADS, stride=a_dh), :]
                                 for t in range(NT)], axis=1) for d in range(a_dh)]
        return pltpu.bitcast(jnp.concatenate(rows, axis=0).astype(BF16), U32)

    def a_view(n):
        return qkvo_v.at[:, :, pl.ds(pl.multiple_of(n * A_ROWS, A_ROWS), A_HALO + A_ROWS), :]

    def a_project(n):
        x = ax_v[pl.ds(pl.multiple_of(n * A_ROWS, A_ROWS), A_ROWS), :]
        buf = a_view(n)

        def piece(m, j):
            w = wqkv_p[m, j * LANES // 2:(j + 1) * LANES // 2, :]
            buf[m, j, A_HALO:, :] = _dot(x, pltpu.bitcast(w, BF16), _NT)
        return [functools.partial(piece, m, j) for m in range(3) for j in range(NT)]

    def a_attend(n, first=False):
        buf = a_view(n)
        val = {}
        tap = lambda m, j, b0, w: buf[m, j, pl.ds(A_HALO + b0 - w * A_DIL, A_SUB), :]

        def products(b0):
            q = [tap(0, j, b0, 0) for j in range(NT)]
            ts = [functools.reduce(jnp.add, [q[j] * tap(1, j, b0, w) for j in range(NT)])
                  for w in range(A_TAPS)]
            val[b0] = [(t, pltpu.roll(t, 2 * A_HEADS, 1)) for t in ts]

        def fold(b0):
            ts = [t + r for t, r in val[b0]]
            val[b0] = [(t, pltpu.roll(t, A_HEADS, 1)) for t in ts]

        def combine(b0):
            logits = [(t + r) * a_scale for t, r in val.pop(b0)]
            for w in range(A_TAPS):
                if first and b0 < w * A_DIL:
                    pos = b0 + lax.broadcasted_iota(jnp.int32, (A_SUB, LANES), 0)
                    logits[w] = jnp.where(pos >= w * A_DIL, logits[w], NEG)
            mx = functools.reduce(jnp.maximum, logits)
            es = [jnp.exp(t - mx) for t in logits]
            inv = 1.0 / functools.reduce(jnp.add, es)
            for j in range(NT):
                o = functools.reduce(jnp.add, [es[w] * tap(2, j, b0, w) for w in range(A_TAPS)])
                buf[3, j, pl.ds(A_HALO + b0, A_SUB), :] = o * inv

        starts = list(range(0, A_ROWS, A_SUB))
        stages = (products, fold, combine)

        def piece(i):
            for lag, stage in reversed(list(enumerate(stages))):
                if 0 <= i - lag < len(starts):
                    stage(starts[i - lag])
        return [functools.partial(piece, i) for i in range(len(starts) + len(stages) - 1)]

    def a_output(n):
        r0 = pl.multiple_of(n * A_ROWS, A_ROWS)
        buf = a_view(n)

        def piece(j):
            cols = slice(j * LANES, (j + 1) * LANES)
            o = jnp.concatenate([buf[3, t, A_HALO:, :] for t in range(NT)], axis=1)
            outa_v[pl.ds(r0, A_ROWS), cols] = _dot(
                o, pltpu.bitcast(awo_p[:, cols], BF16)).astype(BF16)
        return [functools.partial(piece, j) for j in range(NT)]

    cp_wqkv.start()
    cp_ax(0).start()
    cp_awo.start()
    cp_wqkv.wait()
    cp_ax(1).start()
    cp_ax(2).start()
    for c in range(W_AHEAD - 1):
        start_wt(c)
    cp_bx0.start()
    for j in range(3):
        wqkv_p[j] = permute_rows(j, wqkv_v[:, j * D:(j + 1) * D].T)
    cp_awo.wait()
    awo_p[...] = permute_rows(3, awo_v[...])
    cp_ax(0).wait()
    _interleave(a_project(0))
    cp_ax(3).start()
    start_wt(W_AHEAD - 1)
    cp_ax(1).wait()
    for m in (1, 2):
        for j in range(NT):
            qkvo_v[m, j, 0:A_HALO, :] = jnp.broadcast_to(
                qkvo_v[m, j, A_HALO:A_HALO + 1, :], (A_HALO, LANES))
    _interleave(a_project(1), a_attend(0, first=True))

    def a_iter(i, carry):
        pl.when(i + 4 < n_blk)(lambda: cp_ax(i + 4).start())
        pl.when(i + W_AHEAD < n_blk)(lambda: start_wt(i + W_AHEAD))
        for c, at in enumerate(BWO_START):
            if at < n_blk - 2:
                pl.when(i == at)(cp_bwo(c).start)
        cp_ax(i + 2).wait()
        wait_wt(i)
        _interleave(a_project(i + 2), a_output(i), a_attend(i + 1), transpose_wt(i))
        return carry

    lax.fori_loop(0, n_blk - 2, a_iter, 0)

    b_scale = DH ** -0.5
    schedule = _b_schedule(n_pairs)

    def b_step(s, mem, before=None):
        lane = lax.broadcasted_iota(jnp.int32, (L, PW), 1)
        lo = lane < DH
        row = lax.broadcasted_iota(jnp.int32, (L, 2 * L), 0)
        col = lax.broadcasted_iota(jnp.int32, (L, 2 * L), 1)
        in0 = col < L
        visible = (row < M) | (row >= jnp.where(in0, col, col - L))

        def split_heads(t):
            return jnp.concatenate(
                [jnp.where(lo, t, 0.0), jnp.where(lo, 0.0, t)], axis=0).astype(BF16)

        def proj(m, p):
            return _dot(h, pltpu.bitcast(w_v[m, :, p * PW:(p + 1) * PW], BF16))

        r0 = pl.multiple_of(s * seg, seg)
        h = jnp.concatenate([mem, bx_v[pl.ds(r0, seg), :].astype(F32)], axis=0)
        acc = None
        val = {}
        for op, p in schedule:
            if before is not None:
                before(op, p)
            if op == "q":
                val["q", p] = proj(0, p)
            elif op == "k":
                val["k", p] = split_heads(proj(1, p))
            elif op == "v":
                val["v", p] = split_heads(proj(2, p))
            elif op == "s":
                sc = _dot(val.pop(("q", p)), val.pop(("k", p)), _NT) * b_scale
                sc = jnp.where(visible, sc, NEG)
                m0 = jnp.max(jnp.where(in0, sc, -jnp.inf), axis=1, keepdims=True)
                m1 = jnp.max(jnp.where(in0, -jnp.inf, sc), axis=1, keepdims=True)
                e = jnp.exp(sc - jnp.where(in0, m0, m1))
                d0 = jnp.sum(jnp.where(in0, e, 0.0), axis=1, keepdims=True)
                d1 = jnp.sum(jnp.where(in0, 0.0, e), axis=1, keepdims=True)
                val["p", p] = e / jnp.where(in0, d0, d1)
            elif op == "pv":
                val["o", p] = _dot(val.pop(("p", p)), val.pop(("v", p)))
            else:
                t = _dot(val.pop(("o", p)), bwo_v[p * PW:(p + 1) * PW, :])
                acc = t if acc is None else acc + t
        outb_v[pl.ds(r0, seg), :] = acc[M:].astype(BF16)
        cp_outb(s).start()
        return acc[:M].astype(BF16).astype(F32)

    for c, at in enumerate(BWO_START):
        if at == n_blk - 2:
            cp_bwo(c).start()
    wait_wt(n_blk - 2)
    wait_wt(n_blk - 1)
    cp_bx0.wait()
    _interleave(a_output(n_blk - 2))
    side = (a_attend(n_blk - 1) + transpose_wt(n_blk - 2) + transpose_wt(n_blk - 1)
            + a_output(n_blk - 1))
    ready = (n_blk - 2) * CH // PW
    per_op = pl.cdiv(len(side), len([1 for op, p in schedule if op in "qkv" and p < ready]))
    bwo_pairs = n_pairs // len(BWO_START)

    def first_step_hook(op, p):
        if op in "qkv":
            for _ in range(min(per_op, len(side))):
                side.pop(0)()
        if op == "o" and p % bwo_pairs == 0:
            cp_bwo(p // bwo_pairs).wait()

    mem = b_step(0, mem0_ref[...].astype(F32), first_step_hook)
    cp_bx1.start()
    cp_outa.start()

    def b_iter(s, mem):
        pl.when(s == head // seg)(cp_bx1.wait)
        return b_step(s, mem)

    lax.fori_loop(1, n_seg, b_iter, mem)

    cp_outa.wait()
    pltpu.make_async_copy(outb_v, out_hbm.at[:, pl.ds(D, D)], sem_o.at[1]).wait()


@functools.partial(jax.jit, static_argnames=("B_seg_len",))
def pallas_concat_heads__sliding_local_dilated__memory_aug_recurrent_mem_tr__prompt_kernel(
    A_x: jax.Array,
    A_wqkv: jax.Array,
    A_wo: jax.Array,
    B_x: jax.Array,
    B_mem0: jax.Array,
    B_Wq: jax.Array,
    B_Wk: jax.Array,
    B_Wv: jax.Array,
    B_Wo: jax.Array,
    B_seg_len: int,
):
    B, S, D = A_x.shape
    _, H, DH = B_Wq.shape
    M = B_mem0.shape[1]
    HD = H * DH
    NT = D // LANES
    n_blk = S // A_ROWS
    assert B == 1 and B_x.shape == A_x.shape and A_x.dtype == BF16

    wt = lambda w: w.transpose(1, 2, 0).reshape(HD, D)
    hbm = pl.BlockSpec(memory_space=pl.ANY)
    out = pl.pallas_call(
        functools.partial(_kernel, seg=int(B_seg_len), n_heads=H),
        out_shape=jax.ShapeDtypeStruct((S, 2 * D), BF16),
        in_specs=[hbm, hbm, hbm, hbm, pl.BlockSpec(memory_space=pltpu.VMEM),
                  hbm, hbm, hbm, hbm],
        out_specs=hbm,
        scratch_shapes=[
            pltpu.VMEM((S, D), BF16),
            pltpu.VMEM((D, 3 * D), BF16),
            pltpu.VMEM((D, D), BF16),
            pltpu.VMEM((4, NT, D, LANES), F32),
            pltpu.VMEM((3, D // 2, D), U32),
            pltpu.VMEM((D // 2, D), U32),
            pltpu.VMEM((4, NT, A_HALO + S, LANES), F32),
            pltpu.VMEM((S, D), BF16),
            pltpu.VMEM((S, D), BF16),
            pltpu.VMEM((3, HD, D), BF16),
            pltpu.VMEM((3, D // 2, HD), U32),
            pltpu.VMEM((HD, D), BF16),
            pltpu.VMEM((S, D), BF16),
            pltpu.SemaphoreType.DMA((4 + len(BWO_START),)),
            pltpu.SemaphoreType.DMA((4, n_blk)),
            pltpu.SemaphoreType.DMA((2,)),
        ],
        compiler_params=pltpu.CompilerParams(vmem_limit_bytes=112 << 20),
    )(A_x.reshape(S, D), A_wqkv, A_wo, B_x.reshape(S, D), B_mem0.reshape(M, D),
      wt(B_Wq), wt(B_Wk), wt(B_Wv), B_Wo.reshape(HD, D))
    return out.reshape(B, S, 2 * D)
```

```python
import functools

import jax
import jax.numpy as jnp
from jax import lax
from jax.experimental import pallas as pl
from jax.experimental.pallas import tpu as pltpu

F32 = jnp.float32
BF16 = jnp.bfloat16
U32 = jnp.uint32
LANES = 128
NEG = -1000000000.0

_NN = (((1,), (0,)), ((), ()))
_NT = (((1,), (1,)), ((), ()))

A_HEADS = 32
A_TAPS = 8
A_DIL = 2
A_HALO = 16
A_ROWS = 256
A_SUB = 16
W_AHEAD = 3
B_UNROLL = 2
B_LATE = 5
BWO_START = (5, 6)


def _dot(a, b, dims=_NN):
    return lax.dot_general(a, b, dims, preferred_element_type=F32)


def _interleave(*streams):
    order = [((i + 0.5) / len(st), k, i) for k, st in enumerate(streams) for i in range(len(st))]
    for _, k, i in sorted(order):
        streams[k][i]()


def _b_schedule(n_pairs):
    lag_s, lag_pv, lag_o = 1, 2, 5
    seq = []
    for p in range(n_pairs):
        seq += [("q", p), ("k", p)]
        if p >= lag_s:
            seq.append(("s", p - lag_s))
        seq.append(("v", p))
        if p >= lag_pv:
            seq.append(("pv", p - lag_pv))
        if p >= lag_o:
            seq.append(("o", p - lag_o))
    n = n_pairs
    seq += [("s", n - 1), ("o", n - 5), ("pv", n - 2), ("o", n - 4), ("o", n - 3),
            ("pv", n - 1), ("o", n - 2), ("o", n - 1)]
    return seq


def _kernel(ax_hbm, wqkv_hbm, awo_hbm, bx_hbm, mem0_ref, wqt_hbm, wkt_hbm, wvt_hbm,
            bwo_hbm, out_hbm,
            ax_v, wqkv_v, awo_v, perm_v, wqkv_p, awo_p, qkvo_v, outa_v,
            bx_v, wt_v, w_v, bwo_v, outb_v,
            sem_a, sem_w, sem_o, *, seg, n_heads):
    S, D = ax_v.shape
    NT = D // LANES
    n_blk = S // A_ROWS
    HD = bwo_hbm.shape[0]
    DH = HD // n_heads
    PW = 2 * DH
    n_pairs = n_heads // 2
    M = mem0_ref.shape[0]
    L = M + seg
    n_seg = S // seg
    CH = HD // n_blk
    w_hbm = (wqt_hbm, wkt_hbm, wvt_hbm)

    head = (1 + B_UNROLL) * seg
    cp_wqkv = pltpu.make_async_copy(wqkv_hbm, wqkv_v, sem_a.at[0])
    cp_awo = pltpu.make_async_copy(awo_hbm, awo_v, sem_a.at[1])
    cp_bx0 = pltpu.make_async_copy(bx_hbm.at[pl.ds(0, head), :], bx_v.at[pl.ds(0, head), :],
                                   sem_a.at[2])
    cp_bx1 = pltpu.make_async_copy(bx_hbm.at[pl.ds(head, S - head), :],
                                   bx_v.at[pl.ds(head, S - head), :], sem_a.at[3])
    cp_outa = pltpu.make_async_copy(outa_v, out_hbm.at[:, pl.ds(0, D)], sem_o.at[0])

    def rows_copy(src, dst, rows, c, sem):
        r0 = pl.multiple_of(c * rows, rows)
        return pltpu.make_async_copy(src.at[pl.ds(r0, rows), :], dst.at[pl.ds(r0, rows), :], sem)

    cp_wt = lambda m, c: rows_copy(w_hbm[m], wt_v.at[m], CH, c, sem_w.at[m, c])
    cp_bwo = lambda c: rows_copy(bwo_hbm, bwo_v, HD // len(BWO_START), c, sem_a.at[4 + c])
    cp_ax = lambda c: rows_copy(ax_hbm, ax_v, A_ROWS, c, sem_w.at[3, c])

    def cp_outb(s, n):
        rows = pl.ds(pl.multiple_of(s * seg, seg), n * seg)
        return pltpu.make_async_copy(outb_v.at[rows, :], out_hbm.at[rows, pl.ds(D, D)],
                                     sem_o.at[1])

    def start_wt(c):
        for m in range(3):
            cp_wt(m, c).start()

    def wait_wt(c):
        for m in range(3):
            cp_wt(m, c).wait()

    def transpose_wt(c):
        def piece(m, t):
            c0 = pl.multiple_of(c * CH + t * LANES, LANES)
            w_v[m, :, pl.ds(c0, LANES)] = pltpu.bitcast(wt_v[m, pl.ds(c0, LANES), :].T, U32)
        return [functools.partial(piece, m, t) for t in range(CH // LANES) for m in range(3)]

    a_dh = D // A_HEADS
    a_scale = a_dh ** -0.5

    def permute_rows(j, rows):
        rows = rows.astype(F32)
        for t in range(NT):
            perm_v[j, t] = rows[:, t * LANES:(t + 1) * LANES]
        rows = [jnp.concatenate([perm_v[j, t, pl.ds(d, A_HEADS, stride=a_dh), :]
                                 for t in range(NT)], axis=1) for d in range(a_dh)]
        return pltpu.bitcast(jnp.concatenate(rows, axis=0).astype(BF16), U32)

    def a_view(n):
        return qkvo_v.at[:, :, pl.ds(pl.multiple_of(n * A_ROWS, A_ROWS), A_HALO + A_ROWS), :]

    def a_project(n):
        x = ax_v[pl.ds(pl.multiple_of(n * A_ROWS, A_ROWS), A_ROWS), :]
        buf = a_view(n)

        def piece(m, j):
            w = wqkv_p[m, j * LANES // 2:(j + 1) * LANES // 2, :]
            buf[m, j, A_HALO:, :] = _dot(x, pltpu.bitcast(w, BF16), _NT)
        return [functools.partial(piece, m, j) for m in range(3) for j in range(NT)]

    def a_attend(n, first=False):
        buf = a_view(n)
        val = {}
        tap = lambda m, j, b0, w: buf[m, j, pl.ds(A_HALO + b0 - w * A_DIL, A_SUB), :]

        def products(b0):
            q = [tap(0, j, b0, 0) for j in range(NT)]
            ts = [functools.reduce(jnp.add, [q[j] * tap(1, j, b0, w) for j in range(NT)])
                  for w in range(A_TAPS)]
            val[b0] = [(t, pltpu.roll(t, 2 * A_HEADS, 1)) for t in ts]

        def fold(b0):
            ts = [t + r for t, r in val[b0]]
            val[b0] = [(t, pltpu.roll(t, A_HEADS, 1)) for t in ts]

        def combine(b0):
            logits = [(t + r) * a_scale for t, r in val.pop(b0)]
            for w in range(A_TAPS):
                if first and b0 < w * A_DIL:
                    pos = b0 + lax.broadcasted_iota(jnp.int32, (A_SUB, LANES), 0)
                    logits[w] = jnp.where(pos >= w * A_DIL, logits[w], NEG)
            mx = functools.reduce(jnp.maximum, logits)
            es = [jnp.exp(t - mx) for t in logits]
            inv = 1.0 / functools.reduce(jnp.add, es)
            for j in range(NT):
                o = functools.reduce(jnp.add, [es[w] * tap(2, j, b0, w) for w in range(A_TAPS)])
                buf[3, j, pl.ds(A_HALO + b0, A_SUB), :] = o * inv

        starts = list(range(0, A_ROWS, A_SUB))
        stages = (products, fold, combine)

        def piece(i):
            for lag, stage in reversed(list(enumerate(stages))):
                if 0 <= i - lag < len(starts):
                    stage(starts[i - lag])
        return [functools.partial(piece, i) for i in range(len(starts) + len(stages) - 1)]

    def a_output(n):
        r0 = pl.multiple_of(n * A_ROWS, A_ROWS)
        buf = a_view(n)

        def piece(j):
            cols = slice(j * LANES, (j + 1) * LANES)
            o = jnp.concatenate([buf[3, t, A_HALO:, :] for t in range(NT)], axis=1)
            outa_v[pl.ds(r0, A_ROWS), cols] = _dot(
                o, pltpu.bitcast(awo_p[:, cols], BF16)).astype(BF16)
        return [functools.partial(piece, j) for j in range(NT)]

    cp_wqkv.start()
    cp_ax(0).start()
    cp_awo.start()
    cp_wqkv.wait()
    cp_ax(1).start()
    cp_ax(2).start()
    for c in range(W_AHEAD - 1):
        start_wt(c)
    cp_bx0.start()
    for j in range(3):
        wqkv_p[j] = permute_rows(j, wqkv_v[:, j * D:(j + 1) * D].T)
    cp_awo.wait()
    awo_p[...] = permute_rows(3, awo_v[...])
    cp_ax(0).wait()
    _interleave(a_project(0))
    cp_ax(3).start()
    start_wt(W_AHEAD - 1)
    cp_ax(1).wait()
    for m in (1, 2):
        for j in range(NT):
            qkvo_v[m, j, 0:A_HALO, :] = jnp.broadcast_to(
                qkvo_v[m, j, A_HALO:A_HALO + 1, :], (A_HALO, LANES))
    _interleave(a_project(1), a_attend(0, first=True))

    def a_iter(i, carry):
        pl.when(i + 4 < n_blk)(lambda: cp_ax(i + 4).start())
        pl.when(i + W_AHEAD < n_blk)(lambda: start_wt(i + W_AHEAD))
        for c, at in enumerate(BWO_START):
            if at < n_blk - 2:
                pl.when(i == at)(cp_bwo(c).start)
        cp_ax(i + 2).wait()
        wait_wt(i)
        _interleave(a_project(i + 2), a_output(i), a_attend(i + 1), transpose_wt(i))
        return carry

    lax.fori_loop(0, n_blk - 2, a_iter, 0)

    b_scale = DH ** -0.5
    schedule = _b_schedule(n_pairs)

    def b_step(s, mem, before=None, last=False):
        q0 = M if last else 0
        lane = lax.broadcasted_iota(jnp.int32, (L, PW), 1)
        lo = lane < DH
        row = q0 + lax.broadcasted_iota(jnp.int32, (L - q0, 2 * L), 0)
        col = lax.broadcasted_iota(jnp.int32, (L - q0, 2 * L), 1)
        in0 = col < L
        visible = (row < M) | (row >= jnp.where(in0, col, col - L))

        def split_heads(t):
            return jnp.concatenate(
                [jnp.where(lo, t, 0.0), jnp.where(lo, 0.0, t)], axis=0).astype(BF16)

        def proj(m, p, k0=0, k1=D):
            w = w_v[m, k0 // 2:k1 // 2, p * PW:(p + 1) * PW]
            return _dot(h[(q0 if m == 0 else 0):, k0:k1], pltpu.bitcast(w, BF16))

        r0 = pl.multiple_of(s * seg, seg)
        h = jnp.concatenate([mem, bx_v[pl.ds(r0, seg), :].astype(F32)], axis=0)
        acc = None
        val = {}
        late = []
        for op, p in schedule:
            if before is not None:
                before(op, p)
            if op == "q" and p == 0:
                q, k = proj(0, 0, 0, D - LANES), proj(1, 0, 0, D - LANES)
                val["q", 0] = proj(0, 0, D - LANES) + q
                val["k", 0] = split_heads(proj(1, 0, D - LANES) + k)
            elif op == "q":
                val["q", p] = proj(0, p)
            elif op == "k":
                if p > 0:
                    val["k", p] = split_heads(proj(1, p))
            elif op == "v":
                val["v", p] = split_heads(proj(2, p))
            elif op == "s":
                sc = _dot(val.pop(("q", p)), val.pop(("k", p)), _NT) * b_scale
                sc = jnp.where(visible, sc, NEG)
                m0 = jnp.max(jnp.where(in0, sc, -jnp.inf), axis=1, keepdims=True)
                m1 = jnp.max(jnp.where(in0, -jnp.inf, sc), axis=1, keepdims=True)
                e = jnp.exp(sc - jnp.where(in0, m0, m1))
                d0 = jnp.sum(jnp.where(in0, e, 0.0), axis=1, keepdims=True)
                d1 = jnp.sum(jnp.where(in0, 0.0, e), axis=1, keepdims=True)
                val["p", p] = e / jnp.where(in0, d0, d1)
            elif op == "pv":
                val["o", p] = _dot(val.pop(("p", p)), val.pop(("v", p)))
            elif p < n_pairs - B_LATE:
                t = _dot(val.pop(("o", p)), bwo_v[p * PW:(p + 1) * PW, :])
                acc = t if acc is None else acc + t
            else:
                if not late:
                    acc, acc_last = acc[:, :D - LANES], acc[:, D - LANES:]
                late.append(val.pop(("o", p)))
                acc = acc + _dot(late[-1], bwo_v[p * PW:(p + 1) * PW, :D - LANES])
        acc_last = acc_last + _dot(jnp.concatenate(late, axis=1),
                                   bwo_v[(n_pairs - B_LATE) * PW:, D - LANES:])
        acc = jnp.concatenate([acc, acc_last], axis=1)
        outb_v[pl.ds(r0, seg), :] = acc[M - q0:].astype(BF16)
        return acc[:M]

    for c, at in enumerate(BWO_START):
        if at == n_blk - 2:
            cp_bwo(c).start()
    wait_wt(n_blk - 2)
    wait_wt(n_blk - 1)
    cp_bx0.wait()
    _interleave(a_output(n_blk - 2))
    side = (a_attend(n_blk - 1) + transpose_wt(n_blk - 2) + transpose_wt(n_blk - 1)
            + a_output(n_blk - 1))
    ready = (n_blk - 2) * CH // PW
    per_op = pl.cdiv(len(side), len([1 for op, p in schedule if op in "qkv" and p < ready]))
    bwo_pairs = n_pairs // len(BWO_START)

    def first_step_hook(op, p):
        if op in "qkv":
            for _ in range(min(per_op, len(side))):
                side.pop(0)()
        if op == "o" and p % bwo_pairs == 0:
            cp_bwo(p // bwo_pairs).wait()

    mem = b_step(0, mem0_ref[...].astype(F32), first_step_hook)
    cp_bx1.start()
    cp_outa.start()
    cp_outb(0, 1).start()

    def b_iter(i, mem):
        pl.when(i == 1)(cp_bx1.wait)
        for u in range(B_UNROLL):
            mem = b_step(1 + i * B_UNROLL + u, mem)
        cp_outb(1 + i * B_UNROLL, B_UNROLL).start()
        return mem

    mem = lax.fori_loop(0, (n_seg - 1) // B_UNROLL, b_iter, mem)
    for s in range(n_seg - (n_seg - 1) % B_UNROLL, n_seg):
        mem = b_step(s, mem, last=s == n_seg - 1)
        cp_outb(s, 1).start()

    cp_outa.wait()
    pltpu.make_async_copy(outb_v, out_hbm.at[:, pl.ds(D, D)], sem_o.at[1]).wait()


@functools.partial(jax.jit, static_argnames=("B_seg_len",))
def pallas_concat_heads__sliding_local_dilated__memory_aug_recurrent_mem_tr__prompt_kernel(
    A_x: jax.Array,
    A_wqkv: jax.Array,
    A_wo: jax.Array,
    B_x: jax.Array,
    B_mem0: jax.Array,
    B_Wq: jax.Array,
    B_Wk: jax.Array,
    B_Wv: jax.Array,
    B_Wo: jax.Array,
    B_seg_len: int,
):
    B, S, D = A_x.shape
    _, H, DH = B_Wq.shape
    M = B_mem0.shape[1]
    HD = H * DH
    NT = D // LANES
    n_blk = S // A_ROWS
    assert B == 1 and B_x.shape == A_x.shape and A_x.dtype == BF16

    wt = lambda w: w.transpose(1, 2, 0).reshape(HD, D)
    hbm = pl.BlockSpec(memory_space=pl.ANY)
    out = pl.pallas_call(
        functools.partial(_kernel, seg=int(B_seg_len), n_heads=H),
        out_shape=jax.ShapeDtypeStruct((S, 2 * D), BF16),
        in_specs=[hbm, hbm, hbm, hbm, pl.BlockSpec(memory_space=pltpu.VMEM),
                  hbm, hbm, hbm, hbm],
        out_specs=hbm,
        scratch_shapes=[
            pltpu.VMEM((S, D), BF16),
            pltpu.VMEM((D, 3 * D), BF16),
            pltpu.VMEM((D, D), BF16),
            pltpu.VMEM((4, NT, D, LANES), F32),
            pltpu.VMEM((3, D // 2, D), U32),
            pltpu.VMEM((D // 2, D), U32),
            pltpu.VMEM((4, NT, A_HALO + S, LANES), F32),
            pltpu.VMEM((S, D), BF16),
            pltpu.VMEM((S, D), BF16),
            pltpu.VMEM((3, HD, D), BF16),
            pltpu.VMEM((3, D // 2, HD), U32),
            pltpu.VMEM((HD, D), BF16),
            pltpu.VMEM((S, D), BF16),
            pltpu.SemaphoreType.DMA((4 + len(BWO_START),)),
            pltpu.SemaphoreType.DMA((4, n_blk)),
            pltpu.SemaphoreType.DMA((2,)),
        ],
        compiler_params=pltpu.CompilerParams(vmem_limit_bytes=112 << 20),
    )(A_x.reshape(S, D), A_wqkv, A_wo, B_x.reshape(S, D), B_mem0.reshape(M, D),
      wt(B_Wq), wt(B_Wk), wt(B_Wv), B_Wo.reshape(HD, D))
    return out.reshape(B, S, 2 * D)
```

```python
import functools

import jax
import jax.numpy as jnp
from jax import lax
from jax.experimental import pallas as pl
from jax.experimental.pallas import tpu as pltpu

F32 = jnp.float32
BF16 = jnp.bfloat16
U32 = jnp.uint32
LANES = 128
NEG = -1000000000.0

_NN = (((1,), (0,)), ((), ()))
_NT = (((1,), (1,)), ((), ()))

A_HEADS = 32
A_TAPS = 8
A_DIL = 2
A_HALO = 16
A_ROWS = 256
A_SUB = 16
W_AHEAD = 3
B_UNROLL = 2
B_LATE = 5
BWO_START = (5, 6)


def _dot(a, b, dims=_NN):
    return lax.dot_general(a, b, dims, preferred_element_type=F32)


def _interleave(*streams):
    order = [((i + 0.5) / len(st), k, i) for k, st in enumerate(streams) for i in range(len(st))]
    for _, k, i in sorted(order):
        streams[k][i]()


def _b_schedule(n_pairs):
    lag_s, lag_pv, lag_o = 1, 2, 5
    seq = []
    for p in range(n_pairs):
        seq += [("q", p), ("k", p)]
        if p >= lag_s:
            seq.append(("s", p - lag_s))
        seq.append(("v", p))
        if p >= lag_pv:
            seq.append(("pv", p - lag_pv))
        if p >= lag_o:
            seq.append(("o", p - lag_o))
    n = n_pairs
    seq += [("s", n - 1), ("o", n - 5), ("pv", n - 2), ("o", n - 4), ("o", n - 3),
            ("pv", n - 1), ("o", n - 2), ("o", n - 1)]
    return seq


def _kernel(ax_hbm, wqkv_hbm, awo_hbm, bx_hbm, mem0_hbm, wqt_hbm, wkt_hbm, wvt_hbm,
            bwo_hbm, out_hbm,
            ax_v, wqkv_v, awo_v, perm_v, wqkv_p, awo_p, qkvo_v, outa_v,
            bx_v, mem0_v, wt_v, w_v, bwo_v, outb_v,
            sem_a, sem_w, sem_o, *, seg, n_heads):
    S, D = ax_v.shape
    NT = D // LANES
    n_blk = S // A_ROWS
    HD = bwo_hbm.shape[0]
    DH = HD // n_heads
    PW = 2 * DH
    n_pairs = n_heads // 2
    M = mem0_v.shape[0]
    L = M + seg
    n_seg = S // seg
    CH = HD // n_blk
    w_hbm = (wqt_hbm, wkt_hbm, wvt_hbm)

    head = (1 + B_UNROLL) * seg
    cp_wqkv = lambda j: pltpu.make_async_copy(wqkv_hbm.at[:, pl.ds(j * D, D)], wqkv_v.at[j],
                                              sem_o.at[2 + j])
    cp_mem0 = pltpu.make_async_copy(mem0_hbm, mem0_v, sem_a.at[0])
    cp_awo = pltpu.make_async_copy(awo_hbm, awo_v, sem_a.at[1])
    cp_bx0 = pltpu.make_async_copy(bx_hbm.at[pl.ds(0, head), :], bx_v.at[pl.ds(0, head), :],
                                   sem_a.at[2])
    cp_bx1 = pltpu.make_async_copy(bx_hbm.at[pl.ds(head, S - head), :],
                                   bx_v.at[pl.ds(head, S - head), :], sem_a.at[3])
    cp_outa = pltpu.make_async_copy(outa_v, out_hbm.at[:, pl.ds(0, D)], sem_o.at[0])

    def rows_copy(src, dst, rows, c, sem):
        r0 = pl.multiple_of(c * rows, rows)
        return pltpu.make_async_copy(src.at[pl.ds(r0, rows), :], dst.at[pl.ds(r0, rows), :], sem)

    cp_wt = lambda m, c: rows_copy(w_hbm[m], wt_v.at[m], CH, c, sem_w.at[m, c])
    cp_bwo = lambda c: rows_copy(bwo_hbm, bwo_v, HD // len(BWO_START), c, sem_a.at[4 + c])
    cp_ax = lambda c: rows_copy(ax_hbm, ax_v, A_ROWS, c, sem_w.at[3, c])

    def cp_outb(s, n):
        rows = pl.ds(pl.multiple_of(s * seg, seg), n * seg)
        return pltpu.make_async_copy(outb_v.at[rows, :], out_hbm.at[rows, pl.ds(D, D)],
                                     sem_o.at[1])

    def start_wt(c):
        for m in range(3):
            cp_wt(m, c).start()

    def wait_wt(c):
        for m in range(3):
            cp_wt(m, c).wait()

    def transpose_wt(c):
        def piece(m, t):
            c0 = pl.multiple_of(c * CH + t * LANES, LANES)
            w_v[m, :, pl.ds(c0, LANES)] = pltpu.bitcast(wt_v[m, pl.ds(c0, LANES), :].T, U32)
        return [functools.partial(piece, m, t) for t in range(CH // LANES) for m in range(3)]

    a_dh = D // A_HEADS
    a_scale = a_dh ** -0.5

    def permute_rows(j, rows):
        rows = rows.astype(F32)
        for t in range(NT):
            perm_v[j, t] = rows[:, t * LANES:(t + 1) * LANES]
        rows = [jnp.concatenate([perm_v[j, t, pl.ds(d, A_HEADS, stride=a_dh), :]
                                 for t in range(NT)], axis=1) for d in range(a_dh)]
        return pltpu.bitcast(jnp.concatenate(rows, axis=0).astype(BF16), U32)

    def a_view(n):
        return qkvo_v.at[:, :, pl.ds(pl.multiple_of(n * A_ROWS, A_ROWS), A_HALO + A_ROWS), :]

    def a_project(n):
        x = ax_v[pl.ds(pl.multiple_of(n * A_ROWS, A_ROWS), A_ROWS), :]
        buf = a_view(n)

        def piece(m, j):
            w = wqkv_p[m, j * LANES // 2:(j + 1) * LANES // 2, :]
            buf[m, j, A_HALO:, :] = _dot(x, pltpu.bitcast(w, BF16), _NT)
        return [functools.partial(piece, m, j) for m in range(3) for j in range(NT)]

    def a_attend(n, first=False):
        buf = a_view(n)
        val = {}
        tap = lambda m, j, b0, w: buf[m, j, pl.ds(A_HALO + b0 - w * A_DIL, A_SUB), :]

        def products(b0):
            q = [tap(0, j, b0, 0) for j in range(NT)]
            ts = [functools.reduce(jnp.add, [q[j] * tap(1, j, b0, w) for j in range(NT)])
                  for w in range(A_TAPS)]
            val[b0] = [(t, pltpu.roll(t, 2 * A_HEADS, 1)) for t in ts]

        def fold(b0):
            ts = [t + r for t, r in val[b0]]
            val[b0] = [(t, pltpu.roll(t, A_HEADS, 1)) for t in ts]

        def combine(b0):
            logits = [(t + r) * a_scale for t, r in val.pop(b0)]
            for w in range(A_TAPS):
                if first and b0 < w * A_DIL:
                    pos = b0 + lax.broadcasted_iota(jnp.int32, (A_SUB, LANES), 0)
                    logits[w] = jnp.where(pos >= w * A_DIL, logits[w], NEG)
            mx = functools.reduce(jnp.maximum, logits)
            es = [jnp.exp(t - mx) for t in logits]
            inv = 1.0 / functools.reduce(jnp.add, es)
            for j in range(NT):
                o = functools.reduce(jnp.add, [es[w] * tap(2, j, b0, w) for w in range(A_TAPS)])
                buf[3, j, pl.ds(A_HALO + b0, A_SUB), :] = o * inv

        starts = list(range(0, A_ROWS, A_SUB))
        stages = (products, fold, combine)

        def piece(i):
            for lag, stage in reversed(list(enumerate(stages))):
                if 0 <= i - lag < len(starts):
                    stage(starts[i - lag])
        return [functools.partial(piece, i) for i in range(len(starts) + len(stages) - 1)]

    def a_output(n):
        r0 = pl.multiple_of(n * A_ROWS, A_ROWS)
        buf = a_view(n)

        def piece(j):
            cols = slice(j * LANES, (j + 1) * LANES)
            o = jnp.concatenate([buf[3, t, A_HALO:, :] for t in range(NT)], axis=1)
            outa_v[pl.ds(r0, A_ROWS), cols] = _dot(
                o, pltpu.bitcast(awo_p[:, cols], BF16)).astype(BF16)
        return [functools.partial(piece, j) for j in range(NT)]

    def permute_wqkv(j):
        wqkv_p[j] = permute_rows(j, wqkv_v[j].T)

    def permute_awo():
        awo_p[...] = permute_rows(3, awo_v[...])

    cp_wqkv(0).start()
    cp_ax(0).start()
    cp_wqkv(1).start()
    cp_wqkv(0).wait()
    permute_wqkv(0)
    cp_wqkv(2).start()
    cp_ax(0).wait()
    cp_wqkv(1).wait()
    cp_ax(1).start()
    cp_awo.start()
    first = a_project(0)
    _interleave(first[:NT], [functools.partial(permute_wqkv, 1)])
    cp_wqkv(2).wait()
    start_wt(0)
    cp_ax(2).start()
    _interleave([functools.partial(permute_wqkv, 2)] + first[NT:])
    cp_ax(1).wait()
    cp_awo.wait()
    cp_ax(3).start()
    for c in range(1, W_AHEAD):
        start_wt(c)
    cp_bx0.start()
    cp_mem0.start()
    for m in (1, 2):
        for j in range(NT):
            qkvo_v[m, j, 0:A_HALO, :] = jnp.broadcast_to(
                qkvo_v[m, j, A_HALO:A_HALO + 1, :], (A_HALO, LANES))
    _interleave(a_project(1), a_attend(0, first=True), [permute_awo])

    def a_iter(i, carry):
        pl.when(i + 4 < n_blk)(lambda: cp_ax(i + 4).start())
        pl.when(i + W_AHEAD < n_blk)(lambda: start_wt(i + W_AHEAD))
        for c, at in enumerate(BWO_START):
            if at < n_blk - 2:
                pl.when(i == at)(cp_bwo(c).start)
        cp_ax(i + 2).wait()
        wait_wt(i)
        _interleave(a_project(i + 2), a_output(i), a_attend(i + 1), transpose_wt(i))
        return carry

    lax.fori_loop(0, n_blk - 2, a_iter, 0)

    b_scale = DH ** -0.5
    schedule = _b_schedule(n_pairs)

    def b_step(s, mem, before=None, last=False):
        q0 = M if last else 0
        lane = lax.broadcasted_iota(jnp.int32, (L, PW), 1)
        lo = lane < DH
        row = q0 + lax.broadcasted_iota(jnp.int32, (L - q0, 2 * L), 0)
        col = lax.broadcasted_iota(jnp.int32, (L - q0, 2 * L), 1)
        in0 = col < L
        visible = (row < M) | (row >= jnp.where(in0, col, col - L))

        def split_heads(t):
            return jnp.concatenate(
                [jnp.where(lo, t, 0.0), jnp.where(lo, 0.0, t)], axis=0).astype(BF16)

        def proj(m, p, k0=0, k1=D):
            w = w_v[m, k0 // 2:k1 // 2, p * PW:(p + 1) * PW]
            return _dot(h[(q0 if m == 0 else 0):, k0:k1], pltpu.bitcast(w, BF16))

        r0 = pl.multiple_of(s * seg, seg)
        h = jnp.concatenate([mem, bx_v[pl.ds(r0, seg), :].astype(F32)], axis=0)
        acc = None
        val = {}
        late = []
        for op, p in schedule:
            if before is not None:
                before(op, p)
            if op == "q" and p == 0:
                q, k = proj(0, 0, 0, D - LANES), proj(1, 0, 0, D - LANES)
                val["q", 0] = proj(0, 0, D - LANES) + q
                val["k", 0] = split_heads(proj(1, 0, D - LANES) + k)
            elif op == "q":
                val["q", p] = proj(0, p)
            elif op == "k":
                if p > 0:
                    val["k", p] = split_heads(proj(1, p))
            elif op == "v":
                val["v", p] = split_heads(proj(2, p))
            elif op == "s":
                sc = _dot(val.pop(("q", p)), val.pop(("k", p)), _NT) * b_scale
                sc = jnp.where(visible, sc, NEG)
                m0 = jnp.max(jnp.where(in0, sc, -jnp.inf), axis=1, keepdims=True)
                m1 = jnp.max(jnp.where(in0, -jnp.inf, sc), axis=1, keepdims=True)
                e = jnp.exp(sc - jnp.where(in0, m0, m1))
                d0 = jnp.sum(jnp.where(in0, e, 0.0), axis=1, keepdims=True)
                d1 = jnp.sum(jnp.where(in0, 0.0, e), axis=1, keepdims=True)
                val["p", p] = e / jnp.where(in0, d0, d1)
            elif op == "pv":
                val["o", p] = _dot(val.pop(("p", p)), val.pop(("v", p)))
            elif p < n_pairs - B_LATE:
                t = _dot(val.pop(("o", p)), bwo_v[p * PW:(p + 1) * PW, :])
                acc = t if acc is None else acc + t
            else:
                if not late:
                    acc, acc_last = acc[:, :D - LANES], acc[:, D - LANES:]
                late.append(val.pop(("o", p)))
                acc = acc + _dot(late[-1], bwo_v[p * PW:(p + 1) * PW, :D - LANES])
        acc_last = acc_last + _dot(jnp.concatenate(late, axis=1),
                                   bwo_v[(n_pairs - B_LATE) * PW:, D - LANES:])
        acc = jnp.concatenate([acc, acc_last], axis=1)
        outb_v[pl.ds(r0, seg), :] = acc[M - q0:].astype(BF16)
        return acc[:M]

    for c, at in enumerate(BWO_START):
        if at == n_blk - 2:
            cp_bwo(c).start()
    wait_wt(n_blk - 2)
    wait_wt(n_blk - 1)
    cp_bx0.wait()
    cp_mem0.wait()
    _interleave(a_output(n_blk - 2))
    side = (a_attend(n_blk - 1) + transpose_wt(n_blk - 2) + transpose_wt(n_blk - 1)
            + a_output(n_blk - 1))
    ready = (n_blk - 2) * CH // PW
    per_op = pl.cdiv(len(side), len([1 for op, p in schedule if op in "qkv" and p < ready]))
    bwo_pairs = n_pairs // len(BWO_START)

    def first_step_hook(op, p):
        if op in "qkv":
            for _ in range(min(per_op, len(side))):
                side.pop(0)()
        if op == "o" and p % bwo_pairs == 0:
            cp_bwo(p // bwo_pairs).wait()

    mem = b_step(0, mem0_v[...].astype(F32), first_step_hook)
    cp_bx1.start()
    cp_outa.start()
    cp_outb(0, 1).start()

    def b_iter(i, mem):
        pl.when(i == 1)(cp_bx1.wait)
        for u in range(B_UNROLL):
            mem = b_step(1 + i * B_UNROLL + u, mem)
        cp_outb(1 + i * B_UNROLL, B_UNROLL).start()
        return mem

    mem = lax.fori_loop(0, (n_seg - 1) // B_UNROLL, b_iter, mem)
    for s in range(n_seg - (n_seg - 1) % B_UNROLL, n_seg):
        mem = b_step(s, mem, last=s == n_seg - 1)
        cp_outb(s, 1).start()

    cp_outa.wait()
    pltpu.make_async_copy(outb_v, out_hbm.at[:, pl.ds(D, D)], sem_o.at[1]).wait()


@functools.partial(jax.jit, static_argnames=("B_seg_len",))
def pallas_concat_heads__sliding_local_dilated__memory_aug_recurrent_mem_tr__prompt_kernel(
    A_x: jax.Array,
    A_wqkv: jax.Array,
    A_wo: jax.Array,
    B_x: jax.Array,
    B_mem0: jax.Array,
    B_Wq: jax.Array,
    B_Wk: jax.Array,
    B_Wv: jax.Array,
    B_Wo: jax.Array,
    B_seg_len: int,
):
    B, S, D = A_x.shape
    _, H, DH = B_Wq.shape
    M = B_mem0.shape[1]
    HD = H * DH
    NT = D // LANES
    n_blk = S // A_ROWS
    assert B == 1 and B_x.shape == A_x.shape and A_x.dtype == BF16

    wt = lambda w: w.transpose(1, 2, 0).reshape(HD, D)
    hbm = pl.BlockSpec(memory_space=pl.ANY)
    out = pl.pallas_call(
        functools.partial(_kernel, seg=int(B_seg_len), n_heads=H),
        out_shape=jax.ShapeDtypeStruct((S, 2 * D), BF16),
        in_specs=[hbm] * 9,
        out_specs=hbm,
        scratch_shapes=[
            pltpu.VMEM((S, D), BF16),
            pltpu.VMEM((3, D, D), BF16),
            pltpu.VMEM((D, D), BF16),
            pltpu.VMEM((4, NT, D, LANES), F32),
            pltpu.VMEM((3, D // 2, D), U32),
            pltpu.VMEM((D // 2, D), U32),
            pltpu.VMEM((4, NT, A_HALO + S, LANES), F32),
            pltpu.VMEM((S, D), BF16),
            pltpu.VMEM((S, D), BF16),
            pltpu.VMEM((M, D), BF16),
            pltpu.VMEM((3, HD, D), BF16),
            pltpu.VMEM((3, D // 2, HD), U32),
            pltpu.VMEM((HD, D), BF16),
            pltpu.VMEM((S, D), BF16),
            pltpu.SemaphoreType.DMA((4 + len(BWO_START),)),
            pltpu.SemaphoreType.DMA((4, n_blk)),
            pltpu.SemaphoreType.DMA((5,)),
        ],
        compiler_params=pltpu.CompilerParams(vmem_limit_bytes=112 << 20),
    )(A_x.reshape(S, D), A_wqkv, A_wo, B_x.reshape(S, D), B_mem0.reshape(M, D),
      wt(B_Wq), wt(B_Wk), wt(B_Wv), B_Wo.reshape(HD, D))
    return out.reshape(B, S, 2 * D)
```

```python
import functools

import jax
import jax.numpy as jnp
from jax import lax
from jax.experimental import pallas as pl
from jax.experimental.pallas import tpu as pltpu

F32 = jnp.float32
BF16 = jnp.bfloat16
U32 = jnp.uint32
LANES = 128
NEG = -1000000000.0

_NN = (((1,), (0,)), ((), ()))
_NT = (((1,), (1,)), ((), ()))

A_HEADS = 32
A_TAPS = 8
A_DIL = 2
A_HALO = 16
A_ROWS = 256
A_SUB = 16
W_AHEAD = 3
B_UNROLL = 2
B_LATE = 5
B_LAG = 5
B_LAG_FIRST = 12
BWO_START = (5, 6)


def _dot(a, b, dims=_NN):
    return lax.dot_general(a, b, dims, preferred_element_type=F32)


def _interleave(*streams):
    order = [((i + 0.5) / len(st), k, i) for k, st in enumerate(streams) for i in range(len(st))]
    for _, k, i in sorted(order):
        streams[k][i]()


def _b_schedule(n, lag_o):
    seq = []
    for p in range(n):
        seq += [("q", p), ("k", p), ("s", p - 1), ("v", p), ("pv", p - 2), ("o", p - lag_o)]
    o = n - lag_o
    seq += [("s", n - 1), ("o", o), ("pv", n - 2), ("o", o + 1), ("o", o + 2), ("pv", n - 1)]
    seq += [("o", p) for p in range(o + 3, n)]
    return [(op, p) for op, p in seq if p >= 0]


def _kernel(ax_hbm, wqkv_hbm, awo_hbm, bx_hbm, mem0_hbm, wqt_hbm, wkt_hbm, wvt_hbm,
            bwo_hbm, out_hbm,
            ax_v, wqkv_v, awo_v, perm_v, wqkv_p, awo_p, qkvo_v, outa_v,
            bx_v, mem0_v, wt_v, w_v, bwo_v, outb_v,
            sem_a, sem_w, sem_o, *, seg, n_heads):
    S, D = ax_v.shape
    NT = D // LANES
    n_blk = S // A_ROWS
    HD = bwo_hbm.shape[0]
    DH = HD // n_heads
    PW = 2 * DH
    n_pairs = n_heads // 2
    M = mem0_v.shape[0]
    L = M + seg
    n_seg = S // seg
    CH = HD // n_blk
    w_hbm = (wqt_hbm, wkt_hbm, wvt_hbm)

    head = (1 + B_UNROLL) * seg
    cp_wqkv = lambda j: pltpu.make_async_copy(wqkv_hbm.at[:, pl.ds(j * D, D)], wqkv_v.at[j],
                                              sem_o.at[2 + j])
    cp_mem0 = pltpu.make_async_copy(mem0_hbm, mem0_v, sem_a.at[0])
    cp_awo = pltpu.make_async_copy(awo_hbm, awo_v, sem_a.at[1])
    cp_bx0 = pltpu.make_async_copy(bx_hbm.at[pl.ds(0, head), :], bx_v.at[pl.ds(0, head), :],
                                   sem_a.at[2])
    cp_bx1 = pltpu.make_async_copy(bx_hbm.at[pl.ds(head, S - head), :],
                                   bx_v.at[pl.ds(head, S - head), :], sem_a.at[3])
    cp_outa = pltpu.make_async_copy(outa_v, out_hbm.at[:, pl.ds(0, D)], sem_o.at[0])

    def rows_copy(src, dst, rows, c, sem):
        r0 = pl.multiple_of(c * rows, rows)
        return pltpu.make_async_copy(src.at[pl.ds(r0, rows), :], dst.at[pl.ds(r0, rows), :], sem)

    cp_wt = lambda m, c: rows_copy(w_hbm[m], wt_v.at[m], CH, c, sem_w.at[m, c])

    def cp_bwo(c):
        split = (n_pairs - B_LATE) * PW
        rows = pl.ds(split, HD - split) if c else pl.ds(0, split)
        return pltpu.make_async_copy(bwo_hbm.at[rows, :], bwo_v.at[rows, :], sem_a.at[4 + c])

    cp_ax = lambda c: rows_copy(ax_hbm, ax_v, A_ROWS, c, sem_w.at[3, c])

    def cp_outb(s, n):
        rows = pl.ds(pl.multiple_of(s * seg, seg), n * seg)
        return pltpu.make_async_copy(outb_v.at[rows, :], out_hbm.at[rows, pl.ds(D, D)],
                                     sem_o.at[1])

    def start_wt(c):
        for m in range(3):
            cp_wt(m, c).start()

    def wait_wt(c):
        for m in range(3):
            cp_wt(m, c).wait()

    def transpose_wt(c):
        def piece(m, t):
            c0 = pl.multiple_of(c * CH + t * LANES, LANES)
            w_v[m, :, pl.ds(c0, LANES)] = pltpu.bitcast(wt_v[m, pl.ds(c0, LANES), :].T, U32)
        return [functools.partial(piece, m, t) for t in range(CH // LANES) for m in range(3)]

    a_dh = D // A_HEADS
    a_scale = a_dh ** -0.5

    def permute_rows(j, rows):
        rows = rows.astype(F32)
        for t in range(NT):
            perm_v[j, t] = rows[:, t * LANES:(t + 1) * LANES]
        rows = [jnp.concatenate([perm_v[j, t, pl.ds(d, A_HEADS, stride=a_dh), :]
                                 for t in range(NT)], axis=1) for d in range(a_dh)]
        return pltpu.bitcast(jnp.concatenate(rows, axis=0).astype(BF16), U32)

    def a_view(n):
        return qkvo_v.at[:, :, pl.ds(pl.multiple_of(n * A_ROWS, A_ROWS), A_HALO + A_ROWS), :]

    def a_project(n):
        x = ax_v[pl.ds(pl.multiple_of(n * A_ROWS, A_ROWS), A_ROWS), :]
        buf = a_view(n)

        def piece(m, j):
            w = wqkv_p[m, j * LANES // 2:(j + 1) * LANES // 2, :]
            buf[m, j, A_HALO:, :] = _dot(x, pltpu.bitcast(w, BF16), _NT)
        return [functools.partial(piece, m, j) for m in range(3) for j in range(NT)]

    def a_attend(n, first=False):
        buf = a_view(n)
        val = {}
        tap = lambda m, j, b0, w: buf[m, j, pl.ds(A_HALO + b0 - w * A_DIL, A_SUB), :]

        def products(b0):
            q = [tap(0, j, b0, 0) for j in range(NT)]
            ts = [functools.reduce(jnp.add, [q[j] * tap(1, j, b0, w) for j in range(NT)])
                  for w in range(A_TAPS)]
            val[b0] = [(t, pltpu.roll(t, 2 * A_HEADS, 1)) for t in ts]

        def fold(b0):
            ts = [t + r for t, r in val[b0]]
            val[b0] = [(t, pltpu.roll(t, A_HEADS, 1)) for t in ts]

        def combine(b0):
            logits = [(t + r) * a_scale for t, r in val.pop(b0)]
            for w in range(A_TAPS):
                if first and b0 < w * A_DIL:
                    pos = b0 + lax.broadcasted_iota(jnp.int32, (A_SUB, LANES), 0)
                    logits[w] = jnp.where(pos >= w * A_DIL, logits[w], NEG)
            mx = functools.reduce(jnp.maximum, logits)
            es = [jnp.exp(t - mx) for t in logits]
            inv = 1.0 / functools.reduce(jnp.add, es)
            for j in range(NT):
                o = functools.reduce(jnp.add, [es[w] * tap(2, j, b0, w) for w in range(A_TAPS)])
                buf[3, j, pl.ds(A_HALO + b0, A_SUB), :] = o * inv

        starts = list(range(0, A_ROWS, A_SUB))
        stages = (products, fold, combine)

        def piece(i):
            for lag, stage in reversed(list(enumerate(stages))):
                if 0 <= i - lag < len(starts):
                    stage(starts[i - lag])
        return [functools.partial(piece, i) for i in range(len(starts) + len(stages) - 1)]

    def a_output(n):
        r0 = pl.multiple_of(n * A_ROWS, A_ROWS)
        buf = a_view(n)

        def piece(j):
            cols = slice(j * LANES, (j + 1) * LANES)
            o = jnp.concatenate([buf[3, t, A_HALO:, :] for t in range(NT)], axis=1)
            outa_v[pl.ds(r0, A_ROWS), cols] = _dot(
                o, pltpu.bitcast(awo_p[:, cols], BF16)).astype(BF16)
        return [functools.partial(piece, j) for j in range(NT)]

    def permute_wqkv(j):
        wqkv_p[j] = permute_rows(j, wqkv_v[j].T)

    def permute_awo():
        awo_p[...] = permute_rows(3, awo_v[...])

    cp_wqkv(0).start()
    cp_ax(0).start()
    cp_wqkv(1).start()
    cp_wqkv(0).wait()
    permute_wqkv(0)
    cp_wqkv(2).start()
    cp_ax(0).wait()
    cp_wqkv(1).wait()
    cp_ax(1).start()
    cp_awo.start()
    first = a_project(0)
    _interleave(first[:NT], [functools.partial(permute_wqkv, 1)])
    cp_wqkv(2).wait()
    start_wt(0)
    cp_ax(2).start()
    _interleave([functools.partial(permute_wqkv, 2)] + first[NT:])
    cp_ax(1).wait()
    cp_awo.wait()
    cp_ax(3).start()
    for c in range(1, W_AHEAD):
        start_wt(c)
    cp_bx0.start()
    cp_mem0.start()
    for m in (1, 2):
        for j in range(NT):
            qkvo_v[m, j, 0:A_HALO, :] = jnp.broadcast_to(
                qkvo_v[m, j, A_HALO:A_HALO + 1, :], (A_HALO, LANES))
    _interleave(a_project(1), a_attend(0, first=True), [permute_awo])

    def a_iter(i, carry):
        pl.when(i + 4 < n_blk)(lambda: cp_ax(i + 4).start())
        pl.when(i + W_AHEAD < n_blk)(lambda: start_wt(i + W_AHEAD))
        for c, at in enumerate(BWO_START):
            if at < n_blk - 2:
                pl.when(i == at)(cp_bwo(c).start)
        cp_ax(i + 2).wait()
        wait_wt(i)
        _interleave(a_project(i + 2), a_output(i), a_attend(i + 1), transpose_wt(i))
        return carry

    lax.fori_loop(0, n_blk - 2, a_iter, 0)

    b_scale = DH ** -0.5

    def b_step(s, mem, before=None, last=False):
        q0 = M if last else 0
        lane = lax.broadcasted_iota(jnp.int32, (L, PW), 1)
        lo = lane < DH
        row = q0 + lax.broadcasted_iota(jnp.int32, (L - q0, 2 * L), 0)
        col = lax.broadcasted_iota(jnp.int32, (L - q0, 2 * L), 1)
        in0 = col < L
        visible = (row < M) | (row >= jnp.where(in0, col, col - L))

        def split_heads(t):
            return jnp.concatenate(
                [jnp.where(lo, t, 0.0), jnp.where(lo, 0.0, t)], axis=0).astype(BF16)

        def proj(m, p, k0=0, k1=D):
            w = w_v[m, k0 // 2:k1 // 2, p * PW:(p + 1) * PW]
            return _dot(h[(q0 if m == 0 else 0):, k0:k1], pltpu.bitcast(w, BF16))

        r0 = pl.multiple_of(s * seg, seg)
        h = jnp.concatenate([mem, bx_v[pl.ds(r0, seg), :].astype(F32)], axis=0)
        acc = None
        val = {}
        late = []
        for op, p in _b_schedule(n_pairs, B_LAG if before is None else B_LAG_FIRST):
            if before is not None:
                before(op, p)
            if op == "q" and p == 0:
                q, k = proj(0, 0, 0, D - LANES), proj(1, 0, 0, D - LANES)
                val["q", 0] = proj(0, 0, D - LANES) + q
                val["k", 0] = split_heads(proj(1, 0, D - LANES) + k)
            elif op == "q":
                val["q", p] = proj(0, p)
            elif op == "k":
                if p > 0:
                    val["k", p] = split_heads(proj(1, p))
            elif op == "v":
                val["v", p] = split_heads(proj(2, p))
            elif op == "s":
                sc = _dot(val.pop(("q", p)), val.pop(("k", p)), _NT) * b_scale
                sc = jnp.where(visible, sc, NEG)
                m0 = jnp.max(jnp.where(in0, sc, -jnp.inf), axis=1, keepdims=True)
                m1 = jnp.max(jnp.where(in0, -jnp.inf, sc), axis=1, keepdims=True)
                e = jnp.exp(sc - jnp.where(in0, m0, m1))
                d0 = jnp.sum(jnp.where(in0, e, 0.0), axis=1, keepdims=True)
                d1 = jnp.sum(jnp.where(in0, 0.0, e), axis=1, keepdims=True)
                val["p", p] = e / jnp.where(in0, d0, d1)
            elif op == "pv":
                val["o", p] = _dot(val.pop(("p", p)), val.pop(("v", p)))
            elif p < n_pairs - B_LATE:
                t = _dot(val.pop(("o", p)), bwo_v[p * PW:(p + 1) * PW, :])
                acc = t if acc is None else acc + t
            else:
                if not late:
                    acc, acc_last = acc[:, :D - LANES], acc[:, D - LANES:]
                late.append(val.pop(("o", p)))
                acc = acc + _dot(late[-1], bwo_v[p * PW:(p + 1) * PW, :D - LANES])
        acc_last = acc_last + _dot(jnp.concatenate(late, axis=1),
                                   bwo_v[(n_pairs - B_LATE) * PW:, D - LANES:])
        acc = jnp.concatenate([acc, acc_last], axis=1)
        outb_v[pl.ds(r0, seg), :] = acc[M - q0:].astype(BF16)
        return acc[:M]

    for c, at in enumerate(BWO_START):
        if at == n_blk - 2:
            cp_bwo(c).start()
    wait_wt(n_blk - 2)
    wait_wt(n_blk - 1)
    cp_bx0.wait()
    cp_mem0.wait()
    _interleave(a_output(n_blk - 2))
    side = (a_attend(n_blk - 1) + transpose_wt(n_blk - 2) + transpose_wt(n_blk - 1)
            + a_output(n_blk - 1))
    ready = (n_blk - 2) * CH // PW
    per_op = pl.cdiv(len(side), 3 * ready)

    def first_step_hook(op, p):
        if op in "qkv":
            for _ in range(min(per_op, len(side))):
                side.pop(0)()
        if op == "o" and p in (0, n_pairs - B_LATE):
            cp_bwo(int(p > 0)).wait()

    mem = b_step(0, mem0_v[...].astype(F32), first_step_hook)
    cp_bx1.start()
    cp_outa.start()
    cp_outb(0, 1).start()

    def b_iter(i, mem):
        pl.when(i == 1)(cp_bx1.wait)
        for u in range(B_UNROLL):
            mem = b_step(1 + i * B_UNROLL + u, mem)
        cp_outb(1 + i * B_UNROLL, B_UNROLL).start()
        return mem

    mem = lax.fori_loop(0, (n_seg - 1) // B_UNROLL, b_iter, mem)
    for s in range(n_seg - (n_seg - 1) % B_UNROLL, n_seg):
        mem = b_step(s, mem, last=s == n_seg - 1)
        cp_outb(s, 1).start()

    cp_outa.wait()
    pltpu.make_async_copy(outb_v, out_hbm.at[:, pl.ds(D, D)], sem_o.at[1]).wait()


@functools.partial(jax.jit, static_argnames=("B_seg_len",))
def pallas_concat_heads__sliding_local_dilated__memory_aug_recurrent_mem_tr__prompt_kernel(
    A_x: jax.Array,
    A_wqkv: jax.Array,
    A_wo: jax.Array,
    B_x: jax.Array,
    B_mem0: jax.Array,
    B_Wq: jax.Array,
    B_Wk: jax.Array,
    B_Wv: jax.Array,
    B_Wo: jax.Array,
    B_seg_len: int,
):
    B, S, D = A_x.shape
    _, H, DH = B_Wq.shape
    M = B_mem0.shape[1]
    HD = H * DH
    NT = D // LANES
    n_blk = S // A_ROWS
    assert B == 1 and B_x.shape == A_x.shape and A_x.dtype == BF16

    wt = lambda w: w.transpose(1, 2, 0).reshape(HD, D)
    hbm = pl.BlockSpec(memory_space=pl.ANY)
    out = pl.pallas_call(
        functools.partial(_kernel, seg=int(B_seg_len), n_heads=H),
        out_shape=jax.ShapeDtypeStruct((S, 2 * D), BF16),
        in_specs=[hbm] * 9,
        out_specs=hbm,
        scratch_shapes=[
            pltpu.VMEM((S, D), BF16),
            pltpu.VMEM((3, D, D), BF16),
            pltpu.VMEM((D, D), BF16),
            pltpu.VMEM((4, NT, D, LANES), F32),
            pltpu.VMEM((3, D // 2, D), U32),
            pltpu.VMEM((D // 2, D), U32),
            pltpu.VMEM((4, NT, A_HALO + S, LANES), F32),
            pltpu.VMEM((S, D), BF16),
            pltpu.VMEM((S, D), BF16),
            pltpu.VMEM((M, D), BF16),
            pltpu.VMEM((3, HD, D), BF16),
            pltpu.VMEM((3, D // 2, HD), U32),
            pltpu.VMEM((HD, D), BF16),
            pltpu.VMEM((S, D), BF16),
            pltpu.SemaphoreType.DMA((4 + len(BWO_START),)),
            pltpu.SemaphoreType.DMA((4, n_blk)),
            pltpu.SemaphoreType.DMA((5,)),
        ],
        compiler_params=pltpu.CompilerParams(vmem_limit_bytes=112 << 20),
    )(A_x.reshape(S, D), A_wqkv, A_wo, B_x.reshape(S, D), B_mem0.reshape(M, D),
      wt(B_Wq), wt(B_Wk), wt(B_Wv), B_Wo.reshape(HD, D))
    return out.reshape(B, S, 2 * D)
```

```python
import functools

import jax
import jax.numpy as jnp
from jax import lax
from jax.experimental import pallas as pl
from jax.experimental.pallas import tpu as pltpu

F32 = jnp.float32
BF16 = jnp.bfloat16
U32 = jnp.uint32
LANES = 128
NEG = -1000000000.0

_NN = (((1,), (0,)), ((), ()))
_NT = (((1,), (1,)), ((), ()))

A_HEADS = 32
A_TAPS = 8
A_DIL = 2
A_HALO = 16
A_ROWS = 256
A_SUB = 16
W_AHEAD = 3
B_UNROLL = 2
B_LATE = 4
B_LAG = 5
B_LAG_FIRST = 12
BWO_START = (5, 6)


def _dot(a, b, dims=_NN):
    return lax.dot_general(a, b, dims, preferred_element_type=F32)


def _interleave(*streams):
    order = [((i + 0.5) / len(st), k, i) for k, st in enumerate(streams) for i in range(len(st))]
    for _, k, i in sorted(order):
        streams[k][i]()


def _b_schedule(n, lag_o):
    seq = []
    for p in range(n):
        seq += [("q", p), ("k", p), ("s", p - 1), ("v", p), ("pv", p - 2), ("o", p - lag_o)]
    o = n - lag_o
    seq += [("s", n - 1), ("o", o), ("pv", n - 2), ("o", o + 1), ("o", o + 2), ("pv", n - 1)]
    seq += [("o", p) for p in range(o + 3, n)]
    return [(op, p) for op, p in seq if p >= 0]


def _kernel(ax_hbm, wqkv_hbm, awo_hbm, bx_hbm, mem0_hbm, wqt_hbm, wkt_hbm, wvt_hbm,
            bwo_hbm, out_hbm,
            ax_v, wqkv_v, awo_v, perm_v, wqkv_p, awo_p, qkvo_v, outa_v,
            bx_v, mem0_v, wt_v, w_v, bwo_v, outb_v,
            sem_a, sem_w, sem_o, *, seg, n_heads):
    S, D = ax_v.shape
    NT = D // LANES
    n_blk = S // A_ROWS
    HD = bwo_hbm.shape[0]
    DH = HD // n_heads
    PW = 2 * DH
    n_pairs = n_heads // 2
    M = mem0_v.shape[0]
    L = M + seg
    n_seg = S // seg
    CH = HD // n_blk
    w_hbm = (wqt_hbm, wkt_hbm, wvt_hbm)

    head = (1 + B_UNROLL) * seg
    cp_wqkv = lambda j: pltpu.make_async_copy(wqkv_hbm.at[:, pl.ds(j * D, D)], wqkv_v.at[j],
                                              sem_a.at[6 + j])
    cp_mem0 = pltpu.make_async_copy(mem0_hbm, mem0_v, sem_a.at[0])
    cp_awo = pltpu.make_async_copy(awo_hbm, awo_v, sem_a.at[1])
    cp_bx0 = pltpu.make_async_copy(bx_hbm.at[pl.ds(0, head), :], bx_v.at[pl.ds(0, head), :],
                                   sem_a.at[2])
    cp_bx1 = pltpu.make_async_copy(bx_hbm.at[pl.ds(head, S - head), :],
                                   bx_v.at[pl.ds(head, S - head), :], sem_a.at[3])
    cp_outa = pltpu.make_async_copy(outa_v, out_hbm.at[:, pl.ds(0, D)], sem_o.at[0])

    def rows_copy(src, dst, rows, c, sem):
        r0 = pl.multiple_of(c * rows, rows)
        return pltpu.make_async_copy(src.at[pl.ds(r0, rows), :], dst.at[pl.ds(r0, rows), :], sem)

    cp_wt = lambda m, c: rows_copy(w_hbm[m], wt_v.at[m], CH, c, sem_w.at[m, c])

    def cp_bwo(c):
        split = (n_pairs - B_LATE) * PW
        rows = pl.ds(split, HD - split) if c else pl.ds(0, split)
        return pltpu.make_async_copy(bwo_hbm.at[rows, :], bwo_v.at[rows, :], sem_a.at[4 + c])

    cp_ax = lambda c: rows_copy(ax_hbm, ax_v, A_ROWS, c, sem_w.at[3, c])

    def cp_outb(s, n, sem):
        rows = pl.ds(pl.multiple_of(s * seg, seg), n * seg)
        return pltpu.make_async_copy(outb_v.at[rows, :], out_hbm.at[rows, pl.ds(D, D)],
                                     sem_o.at[sem])

    def start_wt(c):
        for m in range(3):
            cp_wt(m, c).start()

    def wait_wt(c):
        for m in range(3):
            cp_wt(m, c).wait()

    def transpose_wt(c):
        def piece(m, t):
            c0 = pl.multiple_of(c * CH + t * LANES, LANES)
            w_v[m, :, pl.ds(c0, LANES)] = pltpu.bitcast(wt_v[m, pl.ds(c0, LANES), :].T, U32)
        return [functools.partial(piece, m, t) for t in range(CH // LANES) for m in range(3)]

    a_dh = D // A_HEADS
    a_scale = a_dh ** -0.5

    def permute_rows(j, rows):
        rows = rows.astype(F32)
        for t in range(NT):
            perm_v[j, t, 0:D, :] = rows[:, t * LANES:(t + 1) * LANES]
        rows = [jnp.concatenate([perm_v[j, t, pl.ds(d, A_HEADS, stride=a_dh), :]
                                 for t in range(NT)], axis=1) for d in range(a_dh)]
        return pltpu.bitcast(jnp.concatenate(rows, axis=0).astype(BF16), U32)

    def a_view(n):
        return qkvo_v.at[:, :, pl.ds(pl.multiple_of(n * A_ROWS, A_ROWS), A_HALO + A_ROWS), :]

    def a_project(n):
        x = ax_v[pl.ds(pl.multiple_of(n * A_ROWS, A_ROWS), A_ROWS), :]
        buf = a_view(n)

        def piece(m, j):
            w = wqkv_p[m, j * LANES // 2:(j + 1) * LANES // 2, :]
            buf[m, j, A_HALO:, :] = _dot(x, pltpu.bitcast(w, BF16), _NT)
        return [functools.partial(piece, m, j) for m in range(3) for j in range(NT)]

    def a_attend(n, first=False):
        buf = a_view(n)
        val = {}
        tap = lambda m, j, b0, w: buf[m, j, pl.ds(A_HALO + b0 - w * A_DIL, A_SUB), :]

        def products(b0):
            q = [tap(0, j, b0, 0) for j in range(NT)]
            ts = [functools.reduce(jnp.add, [q[j] * tap(1, j, b0, w) for j in range(NT)])
                  for w in range(A_TAPS)]
            val[b0] = [(t, pltpu.roll(t, 2 * A_HEADS, 1)) for t in ts]

        def fold(b0):
            ts = [t + r for t, r in val[b0]]
            val[b0] = [(t, pltpu.roll(t, A_HEADS, 1)) for t in ts]

        def combine(b0):
            logits = [(t + r) * a_scale for t, r in val.pop(b0)]
            for w in range(A_TAPS):
                if first and b0 < w * A_DIL:
                    pos = b0 + lax.broadcasted_iota(jnp.int32, (A_SUB, LANES), 0)
                    logits[w] = jnp.where(pos >= w * A_DIL, logits[w], NEG)
            mx = functools.reduce(jnp.maximum, logits)
            es = [jnp.exp(t - mx) for t in logits]
            inv = 1.0 / functools.reduce(jnp.add, es)
            for j in range(NT):
                o = functools.reduce(jnp.add, [es[w] * tap(2, j, b0, w) for w in range(A_TAPS)])
                buf[3, j, pl.ds(A_HALO + b0, A_SUB), :] = o * inv

        starts = list(range(0, A_ROWS, A_SUB))
        stages = (products, fold, combine)

        def piece(i):
            for lag, stage in reversed(list(enumerate(stages))):
                if 0 <= i - lag < len(starts):
                    stage(starts[i - lag])
        return [functools.partial(piece, i) for i in range(len(starts) + len(stages) - 1)]

    def a_output(n):
        r0 = pl.multiple_of(n * A_ROWS, A_ROWS)
        buf = a_view(n)

        def piece(j):
            cols = slice(j * LANES, (j + 1) * LANES)
            o = jnp.concatenate([buf[3, t, A_HALO:, :] for t in range(NT)], axis=1)
            outa_v[pl.ds(r0, A_ROWS), cols] = _dot(
                o, pltpu.bitcast(awo_p[:, cols], BF16)).astype(BF16)
        return [functools.partial(piece, j) for j in range(NT)]

    def permute_wqkv(j):
        wqkv_p[j] = permute_rows(j, wqkv_v[j].T)

    def permute_awo():
        awo_p[...] = permute_rows(3, awo_v[...])

    cp_wqkv(0).start()
    cp_ax(0).start()
    cp_wqkv(1).start()
    cp_wqkv(0).wait()
    permute_wqkv(0)
    cp_wqkv(2).start()
    cp_ax(0).wait()
    cp_wqkv(1).wait()
    cp_ax(1).start()
    cp_awo.start()
    first = a_project(0)
    _interleave(first[:NT], [functools.partial(permute_wqkv, 1)])
    cp_wqkv(2).wait()
    start_wt(0)
    cp_ax(2).start()
    _interleave([functools.partial(permute_wqkv, 2)] + first[NT:])
    cp_ax(1).wait()
    cp_awo.wait()
    cp_ax(3).start()
    for c in range(1, W_AHEAD):
        start_wt(c)
    cp_bx0.start()
    cp_mem0.start()
    for m in (1, 2):
        for j in range(NT):
            qkvo_v[m, j, 0:A_HALO, :] = jnp.broadcast_to(
                qkvo_v[m, j, A_HALO:A_HALO + 1, :], (A_HALO, LANES))
    _interleave(a_project(1), a_attend(0, first=True), [permute_awo])

    def a_iter(i, carry):
        pl.when(i + 4 < n_blk)(lambda: cp_ax(i + 4).start())
        pl.when(i + W_AHEAD < n_blk)(lambda: start_wt(i + W_AHEAD))
        for c, at in enumerate(BWO_START):
            if at < n_blk - 2:
                pl.when(i == at)(cp_bwo(c).start)
        cp_ax(i + 2).wait()
        wait_wt(i)
        _interleave(a_project(i + 2), a_output(i), a_attend(i + 1), transpose_wt(i))
        return carry

    lax.fori_loop(0, n_blk - 2, a_iter, 0)

    b_scale = DH ** -0.5

    def b_step(s, mem, before=None, last=False):
        q0 = M if last else 0
        lane = lax.broadcasted_iota(jnp.int32, (L, PW), 1)
        lo = lane < DH
        row = q0 + lax.broadcasted_iota(jnp.int32, (L - q0, 2 * L), 0)
        col = lax.broadcasted_iota(jnp.int32, (L - q0, 2 * L), 1)
        in0 = col < L
        visible = (row < M) | (row >= jnp.where(in0, col, col - L))

        def split_heads(t):
            return jnp.concatenate(
                [jnp.where(lo, t, 0.0), jnp.where(lo, 0.0, t)], axis=0).astype(BF16)

        def proj(m, p, k0=0, k1=D):
            w = w_v[m, k0 // 2:k1 // 2, p * PW:(p + 1) * PW]
            return _dot(h[(q0 if m == 0 else 0):, k0:k1], pltpu.bitcast(w, BF16))

        r0 = pl.multiple_of(s * seg, seg)
        h = jnp.concatenate([mem, bx_v[pl.ds(r0, seg), :].astype(F32)], axis=0)
        acc = None
        val = {}
        late = []
        for op, p in _b_schedule(n_pairs, B_LAG if before is None else B_LAG_FIRST):
            if before is not None:
                before(op, p)
            if op == "q" and p == 0:
                q, k = proj(0, 0, 0, D - LANES), proj(1, 0, 0, D - LANES)
                val["q", 0] = proj(0, 0, D - LANES) + q
                val["k", 0] = split_heads(proj(1, 0, D - LANES) + k)
            elif op == "q":
                val["q", p] = proj(0, p)
            elif op == "k":
                if p > 0:
                    val["k", p] = split_heads(proj(1, p))
            elif op == "v":
                val["v", p] = split_heads(proj(2, p))
            elif op == "s":
                sc = _dot(val.pop(("q", p)), val.pop(("k", p)), _NT) * b_scale
                sc = jnp.where(visible, sc, NEG)
                m0 = jnp.max(jnp.where(in0, sc, -jnp.inf), axis=1, keepdims=True)
                m1 = jnp.max(jnp.where(in0, -jnp.inf, sc), axis=1, keepdims=True)
                e = jnp.exp(sc - jnp.where(in0, m0, m1))
                d0 = jnp.sum(jnp.where(in0, e, 0.0), axis=1, keepdims=True)
                d1 = jnp.sum(jnp.where(in0, 0.0, e), axis=1, keepdims=True)
                val["p", p] = e / jnp.where(in0, d0, d1)
            elif op == "pv":
                val["o", p] = _dot(val.pop(("p", p)), val.pop(("v", p)))
            elif p < n_pairs - B_LATE:
                t = _dot(val.pop(("o", p)), bwo_v[p * PW:(p + 1) * PW, :])
                acc = t if acc is None else acc + t
            else:
                if not late:
                    acc, acc_last = acc[:, :D - LANES], acc[:, D - LANES:]
                late.append(val.pop(("o", p)))
                acc = acc + _dot(late[-1], bwo_v[p * PW:(p + 1) * PW, :D - LANES])
        acc_last = acc_last + _dot(jnp.concatenate(late, axis=1),
                                   bwo_v[(n_pairs - B_LATE) * PW:, D - LANES:])
        acc = jnp.concatenate([acc, acc_last], axis=1)
        outb_v[pl.ds(r0, seg), :] = acc[M - q0:].astype(BF16)
        return acc[:M]

    for c, at in enumerate(BWO_START):
        if at == n_blk - 2:
            cp_bwo(c).start()
    wait_wt(n_blk - 2)
    wait_wt(n_blk - 1)
    cp_bx0.wait()
    cp_mem0.wait()
    _interleave(a_output(n_blk - 2))
    side = (a_attend(n_blk - 1) + transpose_wt(n_blk - 2) + transpose_wt(n_blk - 1)
            + a_output(n_blk - 1))
    ready = (n_blk - 2) * CH // PW
    per_op = pl.cdiv(len(side), 3 * ready)

    def first_step_hook(op, p):
        if op in ("q", "k", "v"):
            assert p < ready or not side
            for _ in range(min(per_op, len(side))):
                side.pop(0)()
        if op == "o" and p in (0, n_pairs - B_LATE):
            cp_bwo(int(p > 0)).wait()

    mem = b_step(0, mem0_v[...].astype(F32), first_step_hook)
    cp_bx1.start()
    cp_outa.start()
    cp_outb(0, 1, 1).start()
    cp_iter = lambda i: cp_outb(1 + i * B_UNROLL, B_UNROLL, 2)
    n_iter = (n_seg - 2) // B_UNROLL

    def b_iter(i, mem):
        pl.when(i == 1)(cp_bx1.wait)
        for u in range(B_UNROLL):
            mem = b_step(1 + i * B_UNROLL + u, mem)
        pl.when(i > 0)(lambda: cp_iter(i - 1).wait())
        cp_iter(i).start()
        return mem

    mem = lax.fori_loop(0, n_iter, b_iter, mem)
    b_step(n_seg - 1, mem, last=True)
    cp_outb(n_seg - 1, 1, 3).start()
    cp_outa.wait()
    cp_outb(0, 1, 1).wait()
    cp_iter(n_iter - 1).wait()
    cp_outb(n_seg - 1, 1, 3).wait()


@functools.partial(jax.jit, static_argnames=("B_seg_len",))
def pallas_concat_heads__sliding_local_dilated__memory_aug_recurrent_mem_tr__prompt_kernel(
    A_x: jax.Array,
    A_wqkv: jax.Array,
    A_wo: jax.Array,
    B_x: jax.Array,
    B_mem0: jax.Array,
    B_Wq: jax.Array,
    B_Wk: jax.Array,
    B_Wv: jax.Array,
    B_Wo: jax.Array,
    B_seg_len: int,
):
    B, S, D = A_x.shape
    _, H, DH = B_Wq.shape
    M = B_mem0.shape[1]
    HD = H * DH
    NT = D // LANES
    n_blk = S // A_ROWS
    assert B == 1 and B_x.shape == A_x.shape and A_x.dtype == BF16
    assert LANES == 4 * A_HEADS and D % LANES == 0 and 2 * DH % LANES == 0
    assert 2 * (M + B_seg_len) <= LANES and S % B_seg_len == 0
    assert (S // B_seg_len - 2) % B_UNROLL == 0 and BWO_START[-1] == n_blk - 2

    wt = lambda w: w.transpose(1, 2, 0).reshape(HD, D)
    hbm = pl.BlockSpec(memory_space=pl.ANY)
    out = pl.pallas_call(
        functools.partial(_kernel, seg=int(B_seg_len), n_heads=H),
        out_shape=jax.ShapeDtypeStruct((S, 2 * D), BF16),
        in_specs=[hbm] * 9,
        out_specs=hbm,
        scratch_shapes=[
            pltpu.VMEM((S, D), BF16),
            pltpu.VMEM((3, D, D), BF16),
            pltpu.VMEM((D, D), BF16),
            pltpu.VMEM((4, NT, D + A_HEADS, LANES), F32),
            pltpu.VMEM((3, D // 2, D), U32),
            pltpu.VMEM((D // 2, D), U32),
            pltpu.VMEM((4, NT, A_HALO + S, LANES), F32),
            pltpu.VMEM((S, D), BF16),
            pltpu.VMEM((S, D), BF16),
            pltpu.VMEM((M, D), BF16),
            pltpu.VMEM((3, HD, D), BF16),
            pltpu.VMEM((3, D // 2, HD), U32),
            pltpu.VMEM((HD, D), BF16),
            pltpu.VMEM((S, D), BF16),
            pltpu.SemaphoreType.DMA((9,)),
            pltpu.SemaphoreType.DMA((4, n_blk)),
            pltpu.SemaphoreType.DMA((4,)),
        ],
        compiler_params=pltpu.CompilerParams(vmem_limit_bytes=112 << 20),
    )(A_x.reshape(S, D), A_wqkv, A_wo, B_x.reshape(S, D), B_mem0.reshape(M, D),
      wt(B_Wq), wt(B_Wk), wt(B_Wv), B_Wo.reshape(HD, D))
    return out.reshape(B, S, 2 * D)
```
